```python
import os as _os
_os.environ.setdefault("JAX_PLATFORMS", "cpu")
import jax
import jax.numpy as jnp

def _softmax(x, axis=-1):
    return jax.nn.softmax(x, axis=axis)
def _gelu(x):
    return jax.nn.gelu(x, approximate=True)
def _silu(x):
    return jax.nn.silu(x)
def _sigmoid(x):
    return jax.nn.sigmoid(x)
def _layernorm(x, axis=-1, eps=1e-5):
    m = jnp.mean(x, axis=axis, keepdims=True)
    v = jnp.var(x, axis=axis, keepdims=True)
    return (x - m) / jnp.sqrt(v + eps)
def _scatter_add(tgt, idx, src, axis=0):
    return tgt.at[idx].add(src)
def _segment_sum(src, seg, n):
    return jax.ops.segment_sum(src, seg, n)
class _Rng:
    def __init__(self, key):
        self._k = key
    def _next(self):
        self._k, sub = jax.random.split(self._k)
        return sub
    def normal(self, shape):
        return jax.random.normal(self._next(), shape, dtype=jnp.bfloat16)
    def randint(self, lo, hi, shape):
        return jax.random.randint(self._next(), shape, lo, hi, dtype=jnp.int32)
    def uniform(self, shape, lo=0.0, hi=1.0):
        return jax.random.uniform(self._next(), shape, jnp.bfloat16, lo, hi)
    def permutation(self, n):
        return jax.random.permutation(self._next(), n)


kernel_name = 'sequential_preLN__mha_block__moe_arch_mod__prompt'

def setup_inputs():
    _rng = _Rng(jax.random.key(int.from_bytes(__import__("os").urandom(4), "little")))
    _w = (lambda a: (lambda t: t.astype(jnp.bfloat16) if jnp.issubdtype(t.dtype, jnp.floating) else t)(jnp.asarray(a)))
    def _A_setup():
        B, S, D, H = 1, 2048, 512, 32
        return {
            "x": _w((lambda *s: _rng.normal(s) * 0.05)(B, S, D)),
            "wqkv": _w((lambda *s: _rng.normal(s) * 0.05)(D, 3 * D)),
            "wo": _w((lambda *s: _rng.normal(s) * 0.05)(D, D)),
        }
    _A_in = _A_setup()

    def _B_setup():
        B, S, D, F, C = 1, 2048, 512, 1792, 2
        return {
            "x": _w((lambda *s: _rng.normal(s) * 0.05)(B, S, D)),
            "w_r": _w((lambda *s: _rng.normal(s) * 0.05)(D)),
            "w_gate": _w((lambda *s: _rng.normal(s) * 0.05)(D, F)),
            "w_up": _w((lambda *s: _rng.normal(s) * 0.05)(D, F)),
            "w_down": _w((lambda *s: _rng.normal(s) * 0.05)(F, D)),
        }
    _B_in = _B_setup()

    return {
        "A_x": _A_in["x"],
        "A_wqkv": _A_in["wqkv"],
        "A_wo": _A_in["wo"],
        "B_x": _B_in["x"],
        "B_w_r": _B_in["w_r"],
        "B_w_gate": _B_in["w_gate"],
        "B_w_up": _B_in["w_up"],
        "B_w_down": _B_in["w_down"],
    }

def reference(A_x, A_wqkv, A_wo, B_x, B_w_r, B_w_gate, B_w_up, B_w_down):
    def _A_ref(x, wqkv, wo):
        B, S, D = x.shape
        H = 32
        Dh = D // H
        qkv = (lambda x, *d: x.transpose(*d))((x @ wqkv).reshape(B, S, 3, H, Dh), 2, 0, 3, 1, 4)
        q, k, v = qkv[0], qkv[1], qkv[2]
        scores = jnp.einsum("bhqd,bhkd->bhqk", q, k) * (Dh ** -0.5)
        p = _softmax(scores, axis=-1)
        o = jnp.einsum("bhqk,bhkd->bhqd", p, v)
        return (lambda x, *d: x.transpose(*d))(o, 0, 2, 1, 3).reshape(B, S, D) @ wo

    def _B_ref(x, w_r, w_gate, w_up, w_down):
        B, S, D = x.shape
        C = 2
        r = x @ w_r
        idx = jnp.argsort(-r, axis=-1)[:, :C]
        idx_e = jnp.repeat(idx.reshape(B, C, 1), D, axis=2)
        x_sel = jnp.take_along_axis(x, idx_e, axis=1)
        g = _silu(x_sel @ w_gate)
        u = x_sel @ w_up
        y = (g * u) @ w_down
        r_sel = _sigmoid(jnp.take_along_axis(r, idx, axis=1))
        y = y * r_sel.reshape(B, C, 1)
        b_off = (jnp.arange(B) * S).reshape(B, 1)
        flat_idx = (idx + b_off).reshape(B * C)
        zero = (x * 0.0).reshape(B * S, D)
        upd = _scatter_add(zero, flat_idx, y.reshape(B * C, D), axis=0)
        return x + upd.reshape(B, S, D)

    x = A_x
    h = x + _A_ref(_layernorm(x, axis=-1), A_wqkv, A_wo)
    h2 = h + _B_ref(_layernorm(h, axis=-1), B_w_r, B_w_gate, B_w_up, B_w_down)
    return h2
```

```python
import functools
import jax
import jax.numpy as jnp
from jax import lax
import jax.experimental.pallas as pl
import jax.experimental.pallas.tpu as pltpu

S = 2048
D = 512
H = 32
DH = 16
F = 1792
TQ = 512
NQ = S // TQ
CK = 128
NCK = S // CK
PRO = 8
HPB = 8
SKEW = 2
LAGM = 3
TOTAL = H * NQ
DLAG = NCK + SKEW
TA = 512
NA = S // TA
TC = 256
NC = S // TC
EPS = 1e-5
NEG_BIG = -3.0e38
QSCALE = (DH ** -0.5) * 1.4426950408889634

f32 = jnp.float32
bf16 = jnp.bfloat16
NT = (((1,), (1,)), ((), ()))


def _layernorm(x):
    m = jnp.mean(x, axis=-1, keepdims=True)
    xc = x - m
    v = jnp.mean(xc * xc, axis=-1, keepdims=True)
    return xc * lax.rsqrt(v + EPS)


def _kernel(x_hbm, wqkv_hbm, wo_hbm, wr_ref, wg_hbm, wu_hbm, wd_hbm, out_hbm,
            x_ref, wqkv_ref, wo_ref, wg_ref, wu_ref, wd_ref, wt_ref, ln1_ref,
            k_ref, qt_ref, vt_ref, ot_ref, s0, s1, s2, s3,
            ln2_ref, h_ref, o_ref, r_ref, z_ref, in_sems, out_sems):
    srefs = [s0, s1, s2, s3]

    def x_copy(i):
        return pltpu.make_async_copy(x_hbm.at[pl.ds(i * TA, TA)], x_ref.at[pl.ds(i * TA, TA)], in_sems.at[i])
    w_copies = [
        pltpu.make_async_copy(wqkv_hbm, wqkv_ref, in_sems.at[NA]),
        pltpu.make_async_copy(wo_hbm, wo_ref, in_sems.at[NA + 1]),
        pltpu.make_async_copy(wg_hbm, wg_ref, in_sems.at[NA + 2]),
        pltpu.make_async_copy(wu_hbm, wu_ref, in_sems.at[NA + 3]),
        pltpu.make_async_copy(wd_hbm, wd_ref, in_sems.at[NA + 4]),
    ]
    x_copy(0).start()
    w_copies[0].start()
    for i in range(1, NA):
        x_copy(i).start()
    z_ref[0] = 0

    def ln1(i):
        rows = pl.ds(i * TA, TA)
        ln1_ref[rows, :] = _layernorm(x_ref[rows, :].astype(f32)).astype(bf16)

    x_copy(0).wait()
    ln1(0)
    w_copies[0].wait()
    x_copy(1).wait()
    for c in w_copies[1:]:
        c.start()
    for i in range(NA):
        if 0 < i < NA - 1:
            x_copy(i + 1).wait()
        if i == NA - 1:
            for c in w_copies[1:]:
                c.wait()
        rows = pl.ds(i * TA, TA)
        ln = ln1_ref[rows, :]
        kk = jnp.dot(ln, wqkv_ref[:, D:2 * D], preferred_element_type=f32).astype(bf16)
        for g in range(4):
            k_ref[g, rows, :] = kk[:, g * 128:(g + 1) * 128]
        if i == 0:
            wt_ref[0:D, :] = wqkv_ref[:, 0:D].T
            wt_ref[D:2 * D, :] = wqkv_ref[:, 2 * D:3 * D].T
        if i + 1 < NA:
            ln1(i + 1)
        qv = lax.dot_general(wt_ref[...], ln, NT, preferred_element_type=f32)
        qt = (qv[0:D] * QSCALE).astype(bf16)
        vt = qv[D:2 * D].astype(bf16)
        for b in range(TA // TQ):
            qb = i * (TA // TQ) + b
            qt_ref[qb] = qt[:, b * TQ:(b + 1) * TQ].reshape(4, 128, TQ)
        vt_ref[:, :, rows] = vt.reshape(H, DH, TA)

    def qm_for(t0, hl):
        t = t0 + hl
        qb = t // H
        g = (t % H) // 8
        j = hl % 8
        parts = []
        if j > 0:
            parts.append(jnp.zeros((DH * j, TQ), bf16))
        parts.append(qt_ref[qb, g, j * DH:(j + 1) * DH, :])
        if j < 7:
            parts.append(jnp.zeros((DH * (7 - j), TQ), bf16))
        return jnp.concatenate(parts, axis=0), g

    def slot(n):
        sl = n % (2 * NCK)
        return srefs[sl // 8], (sl % 8) * CK

    def run(t0, n_hi, n_qk, pv_lo, ms, l, acc, extra=None):
        z = z_ref[0]
        ms = dict(ms)
        mx_hist = []
        mx = None
        for n in range(n_hi):
            if extra is not None:
                extra(n)
            if n < n_qk:
                hl, c = divmod(n, NCK)
                if c == 0:
                    qm, g = qm_for(t0, hl)
                sref, off = slot(n)
                s = jnp.dot(k_ref[g, pl.ds(c * CK, CK), :], qm, preferred_element_type=f32)
                sref[pl.ds(off, CK), :] = s
                s3 = s.reshape(CK // 8, 8, TQ)
                for r in range(0, CK // 8, 2):
                    pm = jnp.maximum(s3[r], s3[r + 1])
                    mx = pm if (c == 0 and r == 0) else jnp.maximum(mx, pm)
                mx_hist.append(mx)
                if c == NCK - 1:
                    ms[hl] = jnp.broadcast_to(jnp.max(mx, axis=0, keepdims=True), (8, TQ))
            j = n - DLAG
            if j >= pv_lo:
                hj, cj = divmod(j, NCK)
                tj = t0 + hj
                h = tj % H
                qb = tj // H
                sref, off = slot(j)
                drows = pl.ds(pl.multiple_of(off + z, CK), CK)
                m_eff = ms[hj]
                if n < n_qk and len(mx_hist) > LAGM:
                    m_eff = jnp.maximum(m_eff, jnp.minimum(mx_hist[-1 - LAGM], NEG_BIG))
                p = jnp.exp2(sref[drows, :].reshape(CK // 8, 8, TQ) - m_eff[None])
                for r in range(CK // 8 - 2, -1, -2):
                    pr = p[r + 1] + p[r]
                    l = pr if (cj == 0 and r == CK // 8 - 2) else l + pr
                o = jnp.dot(vt_ref[h, :, pl.ds(cj * CK, CK)], p.reshape(CK, TQ).astype(bf16),
                            preferred_element_type=f32)
                acc = o if cj == 0 else acc + o
                if cj == NCK - 1:
                    lsum = jnp.sum(l, axis=0, keepdims=True)
                    ot_ref[qb, h] = (acc * (1.0 / lsum)).astype(bf16)
        return ms, l, acc

    ms, l, acc = run(0, NCK * PRO, NCK * PRO, 0, {}, None, None)

    def body(i, carry):
        ma, mb, l, acc = carry
        ms, l, acc = run(PRO + HPB * i, NCK * HPB, NCK * HPB, -DLAG, {-2: ma, -1: mb}, l, acc)
        return ms[HPB - 2], ms[HPB - 1], l, acc

    ma, mb, l, acc = lax.fori_loop(0, (TOTAL - PRO) // HPB, body, (ms[PRO - 2], ms[PRO - 1], l, acc))

    def out_copy(i):
        return pltpu.make_async_copy(o_ref.at[pl.ds(i * TC, TC)], out_hbm.at[pl.ds(i * TC, TC)], out_sems.at[i])

    wr16 = jnp.broadcast_to(wr_ref[...].reshape(1, D), (16, D))
    attn = {}
    ln2s = {}

    def c_proj(i):
        qb, part = divmod(i, TQ // TC)
        o_nat = ot_ref[qb, :, :, pl.ds(part * TC, TC)].reshape(D, TC).T
        attn[i] = jnp.dot(o_nat, wo_ref[...], preferred_element_type=f32)

    def c_norm(i):
        rows = pl.ds(i * TC, TC)
        hh = (x_ref[rows, :].astype(f32) + attn.pop(i).astype(bf16).astype(f32)).astype(bf16).astype(f32)
        ln2b = _layernorm(hh).astype(bf16)
        ln2 = ln2b.astype(f32)
        h_ref[rows, :] = hh
        ln2_ref[rows, :] = ln2
        o_ref[rows, :] = (hh + ln2).astype(bf16)
        out_copy(i).start()
        ln2s[i] = ln2b

    def c_route(i):
        rr = lax.dot_general(wr16, ln2s.pop(i), NT, preferred_element_type=f32)
        r_ref[:, pl.ds(i * TC, TC)] = rr[0:8].astype(bf16).astype(f32)

    def extra(n):
        if n % 6 == 0 and n // 6 < 3:
            i = n // 6
            c_proj(i)
            if i >= 1:
                c_norm(i - 1)
            if i >= 2:
                c_route(i - 2)

    run(TOTAL, DLAG, 0, -DLAG, {-2: ma, -1: mb}, l, acc, extra=extra)
    for i in range(3, NC + 2):
        if i < NC:
            c_proj(i)
        if i - 1 < NC:
            c_norm(i - 1)
        c_route(i - 2)

    r = r_ref[0:1, :]
    ids = lax.broadcasted_iota(jnp.int32, (1, S), 1)
    m1 = jnp.max(r)
    i1 = jnp.min(jnp.where(r == m1, ids, S))
    i1 = jnp.minimum(i1, S - 1)
    r2 = jnp.where(ids == i1, -jnp.inf, r)
    m2 = jnp.max(r2)
    i2 = jnp.min(jnp.where((r2 == m2) & (ids != i1), ids, S))
    i2 = jnp.minimum(i2, S - 1)

    rid16 = lax.broadcasted_iota(jnp.int32, (16, D), 0)
    x1 = ln2_ref[pl.ds(i1, 1), :]
    x2 = ln2_ref[pl.ds(i2, 1), :]
    xs = jnp.where(rid16 == 0, x1, jnp.where(rid16 == 1, x2, 0.0))
    xsb = xs.astype(bf16)
    gate = jnp.dot(xsb, wg_ref[...], preferred_element_type=f32)
    up = jnp.dot(xsb, wu_ref[...], preferred_element_type=f32)
    act = (gate * jax.nn.sigmoid(gate) * up).astype(bf16)
    y = jnp.dot(act, wd_ref[...], preferred_element_type=f32)
    rsel = jnp.where(rid16 == 0, m1, m2)
    y = y * jax.nn.sigmoid(rsel)
    for i in range(NC):
        out_copy(i).wait()
    fix = []
    for c, idx in enumerate((i1, i2)):
        base = pl.multiple_of((idx // 16) * 16, 16)
        new_row = h_ref[pl.ds(idx, 1), :] + (xs[c:c + 1] + y[c:c + 1])
        old = o_ref[pl.ds(base, 16), :].astype(f32)
        o_ref[pl.ds(base, 16), :] = jnp.where(rid16 == idx - base, new_row, old).astype(bf16)
        fix.append(base)

    def fix_copy(c):
        return pltpu.make_async_copy(o_ref.at[pl.ds(fix[c], 16)], out_hbm.at[pl.ds(fix[c], 16)], out_sems.at[c])

    fix_copy(0).start()

    @pl.when(fix[0] != fix[1])
    def _():
        fix_copy(1).start()
        fix_copy(1).wait()

    fix_copy(0).wait()


@jax.jit
def pallas_sequential_preLN__mha_block__moe_arch_mod__prompt_kernel(A_x, A_wqkv, A_wo, B_x, B_w_r, B_w_gate, B_w_up, B_w_down):
    del B_x
    x = A_x.reshape(S, D)
    any_spec = pl.BlockSpec(memory_space=pl.ANY)
    out = pl.pallas_call(
        _kernel,
        out_shape=jax.ShapeDtypeStruct((S, D), bf16),
        in_specs=[any_spec, any_spec, any_spec, pl.BlockSpec(memory_space=pltpu.VMEM), any_spec, any_spec, any_spec],
        out_specs=any_spec,
        scratch_shapes=[
            pltpu.VMEM((S, D), bf16),
            pltpu.VMEM((D, 3 * D), bf16),
            pltpu.VMEM((D, D), bf16),
            pltpu.VMEM((D, F), bf16),
            pltpu.VMEM((D, F), bf16),
            pltpu.VMEM((F, D), bf16),
            pltpu.VMEM((2 * D, D), bf16),
            pltpu.VMEM((S, D), bf16),
            pltpu.VMEM((4, S, 128), bf16),
            pltpu.VMEM((NQ, 4, 128, TQ), bf16),
            pltpu.VMEM((H, DH, S), bf16),
            pltpu.VMEM((NQ, H, DH, TQ), bf16),
            pltpu.VMEM((8 * CK, TQ), f32),
            pltpu.VMEM((8 * CK, TQ), f32),
            pltpu.VMEM((8 * CK, TQ), f32),
            pltpu.VMEM((8 * CK, TQ), f32),
            pltpu.VMEM((S, D), f32),
            pltpu.VMEM((S, D), f32),
            pltpu.VMEM((S, D), bf16),
            pltpu.VMEM((8, S), f32),
            pltpu.SMEM((1,), jnp.int32),
            pltpu.SemaphoreType.DMA((NA + 5,)),
            pltpu.SemaphoreType.DMA((NC,)),
        ],
        compiler_params=pltpu.CompilerParams(vmem_limit_bytes=100 * 1024 * 1024),
    )(x, A_wqkv, A_wo, B_w_r, B_w_gate, B_w_up, B_w_down)
    return out.reshape(1, S, D)
```

```python
import jax
import jax.numpy as jnp
from jax import lax
import jax.experimental.pallas as pl
import jax.experimental.pallas.tpu as pltpu

S = 2048
D = 512
H = 32
DH = 16
F = 1792
EPS = 1e-5
QSCALE = (DH ** -0.5) * 1.4426950408889634

TA = 512
NA = S // TA
MQ = 128
TQ = 512
NQ = S // TQ
TOTAL = H * NQ
HPB = 8
CK = 128
NCK = S // CK
DLAG = NCK + 2
TC = 128
NC = S // TC
TO = 256
NO = S // TO

NEG_BIG = -3.0e38
LAGM = 3
PINT = (4, 5, 6, 6)
KB_PER_TILE = (0, 8, 16, 8)
GLAG = 2
PINC = 3
NTAIL = 2
NCOVER = 1

f32 = jnp.float32
bf16 = jnp.bfloat16
NT = (((1,), (1,)), ((), ()))


def _ln_stats(x):
    m = jnp.sum(x, axis=-1, keepdims=True) * (1.0 / D)
    v = jnp.maximum(jnp.sum(x * x, axis=-1, keepdims=True) * (1.0 / D) - m * m, 0.0)
    return m, lax.rsqrt(v + EPS)


def _layernorm(x):
    m = jnp.mean(x, axis=-1, keepdims=True)
    xc = x - m
    v = jnp.mean(xc * xc, axis=-1, keepdims=True)
    return xc * lax.rsqrt(v + EPS)


def _kernel(x_hbm, wqkv_hbm, wo_hbm, wr_hbm, wg_hbm, wu_hbm, wd_hbm, out_hbm,
            x_ref, wqkv_ref, wo_ref, wo32_ref, wr_ref, wg_ref, wu_ref, wd_ref, wt_ref, ln1_ref,
            k_ref, qt_ref, vt_ref, ot_ref, kf_ref, kb_ref, qf_ref, s0, s1, s2, s3,
            ln2_ref, o_ref, z_ref, sems):
    srefs = [s0, s1, s2, s3]

    def x_copy(i):
        return pltpu.make_async_copy(x_hbm.at[pl.ds(i * TA, TA)], x_ref.at[pl.ds(i * TA, TA)],
                                     sems.at[(0, 2, 2, 3)[i]])

    def wqkv_copy(part):
        cols = pl.ds(part * D, D)
        return pltpu.make_async_copy(wqkv_hbm.at[:, cols], wqkv_ref.at[:, cols], sems.at[(3, 1, 3)[part]])

    wo_copy = pltpu.make_async_copy(wo_hbm, wo_ref, sems.at[0])
    late_copies = [
        pltpu.make_async_copy(wr_hbm, wr_ref, sems.at[4]),
        pltpu.make_async_copy(wg_hbm, wg_ref, sems.at[4]),
        pltpu.make_async_copy(wu_hbm, wu_ref, sems.at[4]),
        pltpu.make_async_copy(wd_hbm, wd_ref, sems.at[4]),
    ]
    x_copy(0).start()
    wqkv_copy(1).start()
    for i in range(1, NA):
        x_copy(i).start()
    wqkv_copy(0).start()
    wqkv_copy(2).start()
    z_ref[0] = 0
    for sl in range(2 * NCK - DLAG, 2 * NCK):
        srefs[sl // 8][pl.ds((sl % 8) * CK, CK), :] = jnp.zeros((CK, TQ), f32)

    ln_deps = []

    def ln1(i, pin=False):
        rows = pl.ds(i * TA, TA)
        ln = _layernorm(x_ref[rows, :].astype(f32))
        ln1_ref[rows, :] = ln.astype(bf16)
        if pin:
            for u in range(TA // 8):
                row = ln[8 * u:8 * (u + 1)]
                ln_deps.append(jnp.minimum(jnp.minimum(row[:, 0:128], row[:, 128:256]),
                                           jnp.minimum(row[:, 256:384], row[:, 384:512])))

    jobs = []
    gates = []

    def paced(lhs, with_jobs, n_deps=0):
        if not with_jobs and n_deps == 0:
            return lhs
        n_tiles = (lhs.shape[0] // 16) * (lhs.shape[1] // 128)
        tile_no = 0
        w32 = pltpu.bitcast(lhs, jnp.int32)
        gate = gates[-GLAG] if len(gates) >= GLAG else None
        cols = []
        for kt in range(w32.shape[1] // 128):
            tiles = []
            for u in range(w32.shape[0] // 8):
                tile = w32[8 * u:8 * (u + 1), kt * 128:(kt + 1) * 128]
                lo = None
                src = {}
                tile_no += 1
                for _ in range(n_deps * tile_no // n_tiles - n_deps * (tile_no - 1) // n_tiles):
                    dep = ln_deps.pop(0)
                    lo = dep if lo is None else jnp.minimum(lo, dep)
                for _ in range(KB_PER_TILE[kt] if with_jobs else 0):
                    c, g, lane = jobs.pop(0)
                    if (c, g) not in src:
                        src[c, g] = jnp.where(gate < NEG_BIG, 0.0, kf_ref[c, :, g * 128:(g + 1) * 128])
                    kb = jnp.broadcast_to(src[c, g][:, lane:lane + 1], (8, 128))
                    col = g * 128 + lane
                    kb_ref[col // DH, c, col % DH] = kb
                    lo = kb if lo is None else jnp.minimum(lo, kb)
                tiles.append(tile if lo is None else jnp.where(lo < NEG_BIG, 0, tile))
            cols.append(jnp.concatenate(tiles, axis=0))
        return pltpu.bitcast(jnp.concatenate(cols, axis=1), bf16)

    def proj_k(i):
        for mb in range(TA // MQ):
            r0 = i * TA + mb * MQ
            rows = pl.ds(r0, MQ)
            n_deps = 0 if mb == 0 else -(-len(ln_deps) // (TA // MQ - mb))
            res = jnp.dot(paced(ln1_ref[rows, :], False, n_deps), wqkv_ref[:, D:2 * D],
                          preferred_element_type=f32)
            gates.append(res[0:8, 0:128])
            kk = res.astype(bf16)
            k32 = pltpu.bitcast(kk, jnp.int32)
            for g in range(4):
                k_ref[g, pl.ds(r0 // 2, MQ // 2), :] = k32[:, g * 128:(g + 1) * 128]
            if (r0 + MQ) % (2 * CK) == 0:
                c0 = 2 * (r0 // (2 * CK))
                kf_ref[pl.ds(c0, 2)] = kk[MQ - 16:MQ].astype(f32).reshape(2, 8, D)
                jobs.extend((c, g, lane) for c in (c0, c0 + 1) for g in range(4) for lane in range(128))

    def proj_qv(i):
        rows = pl.ds(i * TA, TA)
        for mb in range(2 * D // MQ):
            r0 = mb * MQ
            wt = paced(wt_ref[pl.ds(r0, MQ), :], True)
            res = lax.dot_general(wt, ln1_ref[rows, :], NT, preferred_element_type=f32)
            gates.append(res[0:8, 0:128])
            if r0 < D:
                qt = (res * QSCALE).astype(bf16)
                qf_ref[pl.ds(i * H + r0 // DH, MQ // DH)] = qt.astype(f32).reshape(MQ // DH, DH, TA)
                qt_ref[i, r0 // 128, pl.ds(r0 % 128, MQ), :] = qt
            else:
                vt_ref[pl.ds((r0 - D) // DH, MQ // DH), :, rows] = (
                    pltpu.bitcast(res.astype(bf16), jnp.int32).reshape(MQ // DH, DH // 2, TA))

    x_copy(0).wait()
    ln1(0)
    wqkv_copy(1).wait()
    proj_k(0)
    x_copy(1).wait()
    x_copy(2).wait()
    ln1(1)
    ln1(2, pin=True)
    proj_k(1)
    x_copy(3).wait()
    wqkv_copy(0).wait()
    wqkv_copy(2).wait()
    wo_copy.start()
    for c in late_copies:
        c.start()
    proj_k(2)
    ln1(3)
    proj_k(3)
    wt_ref[0:D, :] = wqkv_ref[:, 0:D].T
    wt_ref[D:2 * D, :] = wqkv_ref[:, 2 * D:3 * D].T
    for i in range(NA):
        proj_qv(i)
    assert not jobs
    wo_copy.wait()

    def qm_for(t0, hl):
        t = t0 + hl
        qb = t >> 5
        g = (t >> 3) & 3
        j = hl % 8
        parts = []
        if j > 0:
            parts.append(jnp.zeros((DH * j, TQ), bf16))
        parts.append(qt_ref[qb, g, j * DH:(j + 1) * DH, :])
        if j < 7:
            parts.append(jnp.zeros((DH * (7 - j), TQ), bf16))
        return jnp.concatenate(parts, axis=0), g

    def slot(n):
        sl = n % (2 * NCK)
        return srefs[sl // 8], (sl % 8) * CK

    def run(t0, n_hi, n_qk, ms, l, acc, extra=None):
        z = z_ref[0]
        ms = dict(ms)
        mx_hist = []
        mx = None
        mv = None
        for n in range(n_hi):
            if extra is not None:
                extra(n)
            if n < n_qk:
                hl, c = divmod(n, NCK)
                if c == 0:
                    qm, g = qm_for(t0, hl)
                sref, off = slot(n)
                nm = CK - 16 if c % 2 == 1 else CK
                t = t0 + hl
                kbs = [kb_ref[t & (H - 1), c, d] for d in range(DH)]
                cols = []
                for cc in range(TQ // 128):
                    parts = [None, None]
                    for d in range(DH):
                        term = kbs[d] * qf_ref[t, pl.ds(d, 1), cc * 128:(cc + 1) * 128]
                        parts[d % 2] = term if d < 2 else parts[d % 2] + term
                    cols.append(parts[0] + parts[1])
                sv = jnp.concatenate(cols, axis=1)
                sref2, off2 = slot(n | 1)
                sref2[pl.ds(off2 + CK - 16 + 8 * (c % 2), 8), :] = sv
                mv = sv if c == 0 else jnp.maximum(mv, sv)
                k32 = k_ref[g, pl.ds(c * CK // 2, nm // 2), :]
                tiles = [k32[8 * u:8 * (u + 1)] for u in range(nm // 16)]
                for cc, u in enumerate(PINT):
                    tiles[u] = jnp.where(mv[:, cc * 128:(cc + 1) * 128] < NEG_BIG, 0, tiles[u])
                kc = pltpu.bitcast(jnp.concatenate(tiles, axis=0), bf16)
                s = jnp.dot(kc, qm, preferred_element_type=f32)
                sref[pl.ds(off, nm), :] = s
                s3 = s.reshape(nm // 8, 8, TQ)
                for r in range(0, nm // 8, 2):
                    pm = jnp.maximum(s3[r], s3[r + 1])
                    mx = pm if (c == 0 and r == 0) else jnp.maximum(mx, pm)
                mx_hist.append(mx)
                if c == NCK - 1:
                    ms[hl] = jnp.broadcast_to(jnp.max(jnp.maximum(mx, mv), axis=0, keepdims=True), (8, TQ))
            hj, cj = divmod(n - DLAG, NCK)
            tj = t0 + hj
            h = tj & (H - 1)
            sref, off = slot(n - DLAG)
            drows = pl.ds(pl.multiple_of(off + z, CK), CK)
            m_eff = ms[hj]
            if n < n_qk and len(mx_hist) > LAGM:
                m_eff = jnp.maximum(m_eff, jnp.minimum(mx_hist[-1 - LAGM], NEG_BIG))
            p = jnp.exp2(sref[drows, :].reshape(CK // 8, 8, TQ) - m_eff[None])
            for r in range(CK // 8 - 2, -1, -2):
                pr = p[r + 1] + p[r]
                l = pr if (cj == 0 and r == CK // 8 - 2) else l + pr
            o = jnp.dot(pltpu.bitcast(vt_ref[h, :, pl.ds(cj * CK, CK)], bf16), p.reshape(CK, TQ).astype(bf16),
                        preferred_element_type=f32)
            acc = o if cj == 0 else acc + o
            if cj == NCK - 1:
                lsum = jnp.sum(l, axis=0, keepdims=True)
                ot_ref[tj + 2] = (acc * (1.0 / lsum)).astype(bf16)
        return ms, l, acc

    def body(i, carry):
        ma, mb, l, acc = carry
        ms, l, acc = run(HPB * i, NCK * HPB, NCK * HPB, {-2: ma, -1: mb}, l, acc)
        return ms[HPB - 2], ms[HPB - 1], l, acc

    zeros8 = jnp.zeros((8, TQ), f32)
    ma, mb, l, acc = lax.fori_loop(0, TOTAL // HPB, body,
                                   (zeros8, zeros8, zeros8 + 1.0, jnp.zeros((DH, TQ), f32)))

    for c in late_copies:
        c.wait()

    def out_copy(i):
        return pltpu.make_async_copy(o_ref.at[pl.ds(i * TO, TO)], out_hbm.at[pl.ds(i * TO, TO)], sems.at[5])

    wr_row = wr_ref[...].reshape(1, D).astype(f32)
    wr_sum = jnp.sum(wr_row, axis=-1, keepdims=True)
    attn = {}
    deps = {}
    best = []
    int_min = jnp.iinfo(jnp.int32).min
    lane8 = lax.broadcasted_iota(jnp.int32, (8, 128), 1)
    row8 = lax.broadcasted_iota(jnp.int32, (8, 128), 0)

    def make_key(r, ids):
        bits = pltpu.bitcast(r.astype(bf16).astype(f32) + 0.0, jnp.int32)
        return jnp.where(bits >= 0, bits, bits ^ jnp.int32(0x7FFF0000)) | (S - 1 - ids)

    def insert(key):
        if not best:
            best.extend([key, jnp.full((8, 128), int_min, jnp.int32)])
        else:
            lo = jnp.minimum(best[0], key)
            best[0] = jnp.maximum(best[0], key)
            best[1] = jnp.maximum(best[1], lo)

    def all_max(v):
        return jnp.broadcast_to(jnp.max(jnp.max(v, axis=0, keepdims=True), axis=1, keepdims=True), (1, 128))

    def c_proj(i):
        qb, part = divmod(i, TQ // TC)
        o_nat = ot_ref[pl.ds(2 + qb * H, H), :, pl.ds(part * TC, TC)].reshape(D, TC).T
        if i - PINC in deps:
            zero = jnp.where(jnp.concatenate(deps.pop(i - PINC), axis=0) < NEG_BIG, -1, 0)
            head = pltpu.bitcast(pltpu.bitcast(o_nat[:, 0:128], jnp.int32) | zero, bf16)
            o_nat = jnp.concatenate([head, o_nat[:, 128:]], axis=1)
        if i == 1:
            wo32_ref[...] = pltpu.bitcast(wo_ref[...], jnp.int32)
        wo = wo_ref[...] if i == 0 else pltpu.bitcast(wo32_ref[...], bf16)
        attn[i] = jnp.dot(o_nat, wo, preferred_element_type=f32)

    def c_norm(i):
        rows = pl.ds(i * TC, TC)
        hh = x_ref[rows, :].astype(f32) + attn.pop(i)
        m, rstd = _ln_stats(hh)
        ln2 = (hh - m) * rstd
        ln2_ref[rows, :] = ln2.astype(bf16)
        o_ref[rows, :] = (hh + ln2).astype(bf16)
        if ((i + 1) * TC) % TO == 0:
            out_copy((i * TC) // TO).start()
        r = jnp.broadcast_to((jnp.sum(hh * wr_row, axis=-1, keepdims=True) - m * wr_sum) * rstd, (TC, 128))
        if i < NC - NTAIL:
            rc = r[0:8]
            for u in range(1, TC // 8):
                rc = jnp.where(lane8 == u, r[8 * u:8 * (u + 1)], rc)
                if u % 2 == 1:
                    deps.setdefault(i, []).append(rc)
            insert(jnp.where(lane8 < TC // 8, make_key(rc, i * TC + 8 * lane8 + row8), int_min))
            if i == NC - NTAIL - 1:
                k1 = all_max(best[0])
                k2 = all_max(jnp.where(best[0] == k1, best[1], best[0]))
                best[0] = jnp.where(row8 == 0, k1, int_min)
                best[1] = jnp.where(row8 == 0, k2, int_min)
        else:
            for u in range(TC // 8):
                insert(make_key(r[8 * u:8 * (u + 1)], i * TC + 8 * u + row8))

    n_early = (NQ - 1) * (TQ // TC) - NCOVER

    def c_step(i):
        if i < NC:
            c_proj(i)
        if i >= 1:
            c_norm(i - 1)

    def extra(n):
        for i in range(n * n_early // DLAG, (n + 1) * n_early // DLAG):
            c_step(i)

    run(TOTAL, DLAG, 0, {-2: ma, -1: mb}, l, acc, extra=extra)
    for i in range(n_early, NC + 1):
        c_step(i)

    k1 = jnp.max(best[0], axis=0, keepdims=True)
    k2 = jnp.max(jnp.where(best[0] == k1, best[1], best[0]), axis=0, keepdims=True)
    idxs = [S - 1 - (k[0, 0] & (S - 1)) for k in (k1, k2)]
    bases = [pl.multiple_of((idx >> 4) << 4, 16) for idx in idxs]

    xsb = jnp.concatenate([ln2_ref[pl.ds(base, 16), :] for base in bases], axis=0)
    gate = jnp.dot(xsb, wg_ref[...], preferred_element_type=f32)
    up = jnp.dot(xsb, wu_ref[...], preferred_element_type=f32)
    act = (gate * jax.nn.sigmoid(gate) * up).astype(bf16)
    y = jnp.dot(act, wd_ref[...], preferred_element_type=f32)
    rid16 = lax.broadcasted_iota(jnp.int32, (16, D), 0)
    upds = []
    for c, (k, idx, base) in enumerate(zip((k1, k2), idxs, bases)):
        kv = k & jnp.int32(-65536)
        rsel = pltpu.bitcast(jnp.where(kv >= 0, kv, kv ^ jnp.int32(0x7FFF0000)), f32)
        gatew = jnp.concatenate([jax.nn.sigmoid(rsel)] * (D // 128), axis=1)
        upds.append(jnp.where(rid16 == idx - base, y[16 * c:16 * (c + 1)] * gatew, 0.0))
    for i in range(NO):
        out_copy(i).wait()
    for upd, base in zip(upds, bases):
        o_ref[pl.ds(base, 16), :] = (o_ref[pl.ds(base, 16), :].astype(f32) + upd).astype(bf16)

    def fix_copy(c):
        return pltpu.make_async_copy(o_ref.at[pl.ds(bases[c], 16)], out_hbm.at[pl.ds(bases[c], 16)], sems.at[c])

    fix_copy(0).start()

    @pl.when(bases[0] != bases[1])
    def _():
        fix_copy(1).start()
        fix_copy(1).wait()

    fix_copy(0).wait()


@jax.jit
def pallas_sequential_preLN__mha_block__moe_arch_mod__prompt_kernel(
    A_x: jax.Array,
    A_wqkv: jax.Array,
    A_wo: jax.Array,
    B_x: jax.Array,
    B_w_r: jax.Array,
    B_w_gate: jax.Array,
    B_w_up: jax.Array,
    B_w_down: jax.Array,
):
    del B_x
    any_spec = pl.BlockSpec(memory_space=pl.ANY)
    out = pl.pallas_call(
        _kernel,
        out_shape=jax.ShapeDtypeStruct((S, D), bf16),
        in_specs=[any_spec] * 7,
        out_specs=any_spec,
        scratch_shapes=[
            pltpu.VMEM((S, D), bf16),
            pltpu.VMEM((D, 3 * D), bf16),
            pltpu.VMEM((D, D), bf16),
            pltpu.VMEM((D // 2, D), jnp.int32),
            pltpu.VMEM((D,), bf16),
            pltpu.VMEM((D, F), bf16),
            pltpu.VMEM((D, F), bf16),
            pltpu.VMEM((F, D), bf16),
            pltpu.VMEM((2 * D, D), bf16),
            pltpu.VMEM((S, D), bf16),
            pltpu.VMEM((4, S // 2, 128), jnp.int32),
            pltpu.VMEM((NQ, 4, 128, TQ), bf16),
            pltpu.VMEM((H, DH // 2, S), jnp.int32),
            pltpu.VMEM((TOTAL + 2, DH, TQ), bf16),
            pltpu.VMEM((NCK, 8, D), f32),
            pltpu.VMEM((H, NCK, DH, 8, 128), f32),
            pltpu.VMEM((TOTAL, DH, TQ), f32),
            pltpu.VMEM((8 * CK, TQ), f32),
            pltpu.VMEM((8 * CK, TQ), f32),
            pltpu.VMEM((8 * CK, TQ), f32),
            pltpu.VMEM((8 * CK, TQ), f32),
            pltpu.VMEM((S, D), bf16),
            pltpu.VMEM((S, D), bf16),
            pltpu.SMEM((1,), jnp.int32),
            pltpu.SemaphoreType.DMA((6,)),
        ],
        compiler_params=pltpu.CompilerParams(vmem_limit_bytes=110 * 1024 * 1024),
    )(A_x.reshape(S, D), A_wqkv, A_wo, B_w_r, B_w_gate, B_w_up, B_w_down)
    return out.reshape(1, S, D)
```

```python
import jax
import jax.numpy as jnp
from jax import lax
import jax.experimental.pallas as pl
import jax.experimental.pallas.tpu as pltpu

S = 2048
D = 512
H = 32
DH = 16
F = 1792
EPS = 1e-5
QSCALE = (DH ** -0.5) * 1.4426950408889634

TA = 512
NA = S // TA
MQ = 128
TQ = 512
NQ = S // TQ
TOTAL = H * NQ
HPB = 8
CK = 128
NCK = S // CK
DLAG = NCK + 2
TC = 128
NC = S // TC
TO = 256
NO = S // TO

NEG_BIG = -3.0e38
LAGM = 3
PINT = (6, 6, 5, 4)
PSPLIT = 384
KB_PER_TILE = (0, 8, 16, 8)
GLAG = 2
PINC = 3
NTAIL = 2
NCOVER = 1

f32 = jnp.float32
bf16 = jnp.bfloat16
NN = (((1,), (0,)), ((), ()))
NT = (((1,), (1,)), ((), ()))


def _ln_stats(x):
    m = jnp.sum(x, axis=-1, keepdims=True) * (1.0 / D)
    v = jnp.maximum(jnp.sum(x * x, axis=-1, keepdims=True) * (1.0 / D) - m * m, 0.0)
    return m, lax.rsqrt(v + EPS)


def _layernorm(x):
    m = jnp.mean(x, axis=-1, keepdims=True)
    xc = x - m
    v = jnp.mean(xc * xc, axis=-1, keepdims=True)
    return xc * lax.rsqrt(v + EPS)


def _kernel(x_hbm, wqkv_hbm, wo_hbm, wr_hbm, wg_hbm, wu_hbm, wd_hbm, out_hbm,
            x_ref, wqkv_ref, wo_ref, wo32_ref, wr_ref, wg_ref, wu_ref, wd_ref, wt_ref, ln1_ref,
            k_ref, qt_ref, vt_ref, ot_ref, kf_ref, kb_ref, qf_ref, s0, s1, s2, s3,
            ln2_ref, o_ref, z_ref, sems):
    srefs = [s0, s1, s2, s3]

    def x_copy(i):
        return pltpu.make_async_copy(x_hbm.at[pl.ds(i * TA, TA)], x_ref.at[pl.ds(i * TA, TA)],
                                     sems.at[(0, 2, 2, 3)[i]])

    def wqkv_copy(part):
        cols = pl.ds(part * D, D)
        return pltpu.make_async_copy(wqkv_hbm.at[:, cols], wqkv_ref.at[:, cols], sems.at[(3, 1, 3)[part]])

    wo_copy = pltpu.make_async_copy(wo_hbm, wo_ref, sems.at[0])
    late_copies = [
        pltpu.make_async_copy(wr_hbm, wr_ref, sems.at[4]),
        pltpu.make_async_copy(wg_hbm, wg_ref, sems.at[4]),
        pltpu.make_async_copy(wu_hbm, wu_ref, sems.at[4]),
        pltpu.make_async_copy(wd_hbm, wd_ref, sems.at[4]),
    ]
    x_copy(0).start()
    wqkv_copy(1).start()
    for i in range(1, NA):
        x_copy(i).start()
    wqkv_copy(0).start()
    wqkv_copy(2).start()
    z_ref[0] = 0
    for sl in range(2 * NCK - DLAG, 2 * NCK):
        srefs[sl // 8][pl.ds((sl % 8) * CK, CK), :] = jnp.zeros((CK, TQ), f32)

    ln_deps = []

    def ln1(i, pin=False):
        rows = pl.ds(i * TA, TA)
        ln = _layernorm(x_ref[rows, :].astype(f32))
        ln1_ref[rows, :] = ln.astype(bf16)
        if pin:
            for u in range(TA // 8):
                row = ln[8 * u:8 * (u + 1)]
                ln_deps.append(jnp.minimum(jnp.minimum(row[:, 0:128], row[:, 128:256]),
                                           jnp.minimum(row[:, 256:384], row[:, 384:512])))

    jobs = []
    gates = []

    def paced(lhs, with_jobs, n_deps=0):
        if not with_jobs and n_deps == 0:
            return lhs
        n_tiles = (lhs.shape[0] // 16) * (lhs.shape[1] // 128)
        tile_no = 0
        w32 = pltpu.bitcast(lhs, jnp.int32)
        gate = gates[-GLAG] if len(gates) >= GLAG else None
        cols = []
        for kt in range(w32.shape[1] // 128):
            tiles = []
            for u in range(w32.shape[0] // 8):
                tile = w32[8 * u:8 * (u + 1), kt * 128:(kt + 1) * 128]
                lo = None
                src = {}
                tile_no += 1
                for _ in range(n_deps * tile_no // n_tiles - n_deps * (tile_no - 1) // n_tiles):
                    dep = ln_deps.pop(0)
                    lo = dep if lo is None else jnp.minimum(lo, dep)
                for _ in range(KB_PER_TILE[kt] if with_jobs else 0):
                    c, g, lane = jobs.pop(0)
                    if (c, g) not in src:
                        src[c, g] = jnp.where(gate < NEG_BIG, 0.0, kf_ref[c, :, g * 128:(g + 1) * 128])
                    kb = jnp.broadcast_to(src[c, g][:, lane:lane + 1], (8, 128))
                    col = g * 128 + lane
                    kb_ref[col // DH, c, col % DH] = kb
                    lo = kb if lo is None else jnp.minimum(lo, kb)
                tiles.append(tile if lo is None else jnp.where(lo < NEG_BIG, 0, tile))
            cols.append(jnp.concatenate(tiles, axis=0))
        return pltpu.bitcast(jnp.concatenate(cols, axis=1), bf16)

    def proj_k(i):
        for mb in range(TA // MQ):
            r0 = i * TA + mb * MQ
            rows = pl.ds(r0, MQ)
            n_deps = 0 if mb == 0 else -(-len(ln_deps) // (TA // MQ - mb))
            res = jnp.dot(paced(ln1_ref[rows, :], False, n_deps), wqkv_ref[:, D:2 * D],
                          preferred_element_type=f32)
            gates.append(res[0:8, 0:128])
            kk = res.astype(bf16)
            k32 = pltpu.bitcast(kk, jnp.int32)
            for g in range(4):
                k_ref[g, pl.ds(r0 // 2, MQ // 2), :] = k32[:, g * 128:(g + 1) * 128]
            if (r0 + MQ) % (2 * CK) == 0:
                c0 = 2 * (r0 // (2 * CK))
                kf_ref[pl.ds(c0, 2)] = kk[MQ - 16:MQ].astype(f32).reshape(2, 8, D)
                jobs.extend((c, g, lane) for c in (c0, c0 + 1) for g in range(4) for lane in range(128))

    def proj_qv(i):
        rows = pl.ds(i * TA, TA)
        for mb in range(2 * D // MQ):
            r0 = mb * MQ
            wt = paced(wt_ref[pl.ds(r0, MQ), :], True)
            res = lax.dot_general(wt, ln1_ref[rows, :], NT, preferred_element_type=f32)
            gates.append(res[0:8, 0:128])
            if r0 < D:
                qt = (res * QSCALE).astype(bf16)
                qf_ref[pl.ds(i * H + r0 // DH, MQ // DH)] = qt.astype(f32).reshape(MQ // DH, DH, TA)
                qt_ref[i, r0 // 128, pl.ds(r0 % 128, MQ), :] = qt
            else:
                vt_ref[pl.ds((r0 - D) // DH, MQ // DH), :, rows] = (
                    pltpu.bitcast(res.astype(bf16), jnp.int32).reshape(MQ // DH, DH // 2, TA))

    x_copy(0).wait()
    ln1(0)
    wqkv_copy(1).wait()
    proj_k(0)
    x_copy(1).wait()
    x_copy(2).wait()
    ln1(1)
    ln1(2, pin=True)
    proj_k(1)
    x_copy(3).wait()
    wqkv_copy(0).wait()
    wqkv_copy(2).wait()
    wo_copy.start()
    for c in late_copies:
        c.start()
    proj_k(2)
    ln1(3)
    proj_k(3)
    wt_ref[0:D, :] = wqkv_ref[:, 0:D].T
    wt_ref[D:2 * D, :] = wqkv_ref[:, 2 * D:3 * D].T
    for i in range(NA):
        proj_qv(i)
    assert not jobs
    wo_copy.wait()

    def qm_for(t0, hl):
        t = t0 + hl
        qb = t >> 5
        g = (t >> 3) & 3
        j = hl % 8
        parts = []
        if j > 0:
            parts.append(jnp.zeros((DH * j, TQ), bf16))
        parts.append(qt_ref[qb, g, j * DH:(j + 1) * DH, :])
        if j < 7:
            parts.append(jnp.zeros((DH * (7 - j), TQ), bf16))
        return jnp.concatenate(parts, axis=0), g

    def slot(n):
        sl = n % (2 * NCK)
        return srefs[sl // 8], (sl % 8) * CK

    def run(t0, n_hi, n_qk, ms, l, acc, extra=None):
        z = z_ref[0]
        ms = dict(ms)
        mx_hist = []
        mx = None
        mv = None
        for n in range(n_hi):
            if extra is not None:
                extra(n)
            if n < n_qk:
                hl, c = divmod(n, NCK)
                if c == 0:
                    qm, g = qm_for(t0, hl)
                sref, off = slot(n)
                nm = CK - 16 if c % 2 == 1 else CK
                t = t0 + hl
                kbs = [kb_ref[t & (H - 1), c, d] for d in range(DH)]
                cols = []
                for cc in range(TQ // 128):
                    parts = [None, None]
                    for d in range(DH):
                        term = kbs[d] * qf_ref[t, pl.ds(d, 1), cc * 128:(cc + 1) * 128]
                        parts[d % 2] = term if d < 2 else parts[d % 2] + term
                    cols.append(parts[0] + parts[1])
                sv = jnp.concatenate(cols, axis=1)
                sref2, off2 = slot(n | 1)
                sref2[pl.ds(off2 + CK - 16 + 8 * (c % 2), 8), :] = sv
                mv = sv if c == 0 else jnp.maximum(mv, sv)
                k32 = k_ref[g, pl.ds(c * CK // 2, nm // 2), :]
                tiles = [k32[8 * u:8 * (u + 1)] for u in range(nm // 16)]
                for cc, u in enumerate(PINT):
                    tiles[u] = jnp.where(mv[:, cc * 128:(cc + 1) * 128] < NEG_BIG, 0, tiles[u])
                kc = pltpu.bitcast(jnp.concatenate(tiles, axis=0), bf16)
                s = jnp.dot(kc, qm, preferred_element_type=f32)
                sref[pl.ds(off, nm), :] = s
                s3 = s.reshape(nm // 8, 8, TQ)
                for r in range(0, nm // 8, 2):
                    pm = jnp.maximum(s3[r], s3[r + 1])
                    mx = pm if (c == 0 and r == 0) else jnp.maximum(mx, pm)
                mx_hist.append(mx)
                if c == NCK - 1:
                    ms[hl] = jnp.broadcast_to(jnp.max(jnp.maximum(mx, mv), axis=0, keepdims=True), (8, TQ))
            hj, cj = divmod(n - DLAG, NCK)
            tj = t0 + hj
            h = tj & (H - 1)
            sref, off = slot(n - DLAG)
            drows = pl.ds(pl.multiple_of(off + z, CK), CK)
            m_eff = ms[hj]
            if n < n_qk and len(mx_hist) > LAGM:
                m_eff = jnp.maximum(m_eff, jnp.minimum(mx_hist[-1 - LAGM], NEG_BIG))
            p = jnp.exp2(sref[drows, :].reshape(CK // 8, 8, TQ) - m_eff[None])
            for r in range(CK // 8 - 2, -1, -2):
                pr = p[r + 1] + p[r]
                l = pr if (cj == 0 and r == CK // 8 - 2) else l + pr
            vt = pltpu.bitcast(vt_ref[h, :, pl.ds(cj * CK, CK)], bf16)
            p2 = p.reshape(CK, TQ)
            o = jnp.concatenate(
                [lax.dot_general(vt, p2[:, :PSPLIT].astype(bf16), NN, preferred_element_type=f32),
                 lax.dot_general(vt, p2[:, PSPLIT:], NN, preferred_element_type=f32)], axis=1)
            acc = o if cj == 0 else acc + o
            if cj == NCK - 1:
                lsum = jnp.sum(l, axis=0, keepdims=True)
                ot_ref[tj + 2] = (acc * (1.0 / lsum)).astype(bf16)
        return ms, l, acc

    def body(i, carry):
        ma, mb, l, acc = carry
        ms, l, acc = run(HPB * i, NCK * HPB, NCK * HPB, {-2: ma, -1: mb}, l, acc)
        return ms[HPB - 2], ms[HPB - 1], l, acc

    zeros8 = jnp.zeros((8, TQ), f32)
    ma, mb, l, acc = lax.fori_loop(0, TOTAL // HPB, body,
                                   (zeros8, zeros8, zeros8 + 1.0, jnp.zeros((DH, TQ), f32)))

    for c in late_copies:
        c.wait()

    def out_copy(i):
        return pltpu.make_async_copy(o_ref.at[pl.ds(i * TO, TO)], out_hbm.at[pl.ds(i * TO, TO)], sems.at[5])

    wr_row = wr_ref[...].reshape(1, D).astype(f32)
    wr_sum = jnp.sum(wr_row, axis=-1, keepdims=True)
    attn = {}
    deps = {}
    best = []
    int_min = jnp.iinfo(jnp.int32).min
    lane8 = lax.broadcasted_iota(jnp.int32, (8, 128), 1)
    row8 = lax.broadcasted_iota(jnp.int32, (8, 128), 0)

    def make_key(r, ids):
        bits = pltpu.bitcast(r.astype(bf16).astype(f32) + 0.0, jnp.int32)
        return jnp.where(bits >= 0, bits, bits ^ jnp.int32(0x7FFF0000)) | (S - 1 - ids)

    def insert(key):
        if not best:
            best.extend([key, jnp.full((8, 128), int_min, jnp.int32)])
        else:
            lo = jnp.minimum(best[0], key)
            best[0] = jnp.maximum(best[0], key)
            best[1] = jnp.maximum(best[1], lo)

    def all_max(v):
        return jnp.broadcast_to(jnp.max(jnp.max(v, axis=0, keepdims=True), axis=1, keepdims=True), (1, 128))

    def c_proj(i):
        qb, part = divmod(i, TQ // TC)
        o_nat = ot_ref[pl.ds(2 + qb * H, H), :, pl.ds(part * TC, TC)].reshape(D, TC).T
        if i - PINC in deps:
            zero = jnp.where(jnp.concatenate(deps.pop(i - PINC), axis=0) < NEG_BIG, -1, 0)
            head = pltpu.bitcast(pltpu.bitcast(o_nat[:, 0:128], jnp.int32) | zero, bf16)
            o_nat = jnp.concatenate([head, o_nat[:, 128:]], axis=1)
        if i == 1:
            wo32_ref[...] = pltpu.bitcast(wo_ref[...], jnp.int32)
        wo = wo_ref[...] if i == 0 else pltpu.bitcast(wo32_ref[...], bf16)
        attn[i] = jnp.dot(o_nat, wo, preferred_element_type=f32)

    def c_norm(i):
        rows = pl.ds(i * TC, TC)
        hh = x_ref[rows, :].astype(f32) + attn.pop(i)
        m, rstd = _ln_stats(hh)
        ln2 = (hh - m) * rstd
        ln2_ref[rows, :] = ln2.astype(bf16)
        o_ref[rows, :] = (hh + ln2).astype(bf16)
        if ((i + 1) * TC) % TO == 0:
            out_copy((i * TC) // TO).start()
        r = jnp.broadcast_to((jnp.sum(hh * wr_row, axis=-1, keepdims=True) - m * wr_sum) * rstd, (TC, 128))
        if i < NC - NTAIL:
            rc = r[0:8]
            for u in range(1, TC // 8):
                rc = jnp.where(lane8 == u, r[8 * u:8 * (u + 1)], rc)
                if u % 2 == 1:
                    deps.setdefault(i, []).append(rc)
            insert(jnp.where(lane8 < TC // 8, make_key(rc, i * TC + 8 * lane8 + row8), int_min))
            if i == NC - NTAIL - 1:
                k1 = all_max(best[0])
                k2 = all_max(jnp.where(best[0] == k1, best[1], best[0]))
                best[0] = jnp.where(row8 == 0, k1, int_min)
                best[1] = jnp.where(row8 == 0, k2, int_min)
        else:
            for u in range(TC // 8):
                insert(make_key(r[8 * u:8 * (u + 1)], i * TC + 8 * u + row8))

    n_early = (NQ - 1) * (TQ // TC) - NCOVER

    def c_step(i):
        if i < NC:
            c_proj(i)
        if i >= 1:
            c_norm(i - 1)

    def extra(n):
        for i in range(n * n_early // DLAG, (n + 1) * n_early // DLAG):
            c_step(i)

    run(TOTAL, DLAG, 0, {-2: ma, -1: mb}, l, acc, extra=extra)
    for i in range(n_early, NC + 1):
        c_step(i)

    k1 = jnp.max(best[0], axis=0, keepdims=True)
    k2 = jnp.max(jnp.where(best[0] == k1, best[1], best[0]), axis=0, keepdims=True)
    idxs = [S - 1 - (k[0, 0] & (S - 1)) for k in (k1, k2)]
    bases = [pl.multiple_of((idx >> 4) << 4, 16) for idx in idxs]

    xsb = jnp.concatenate([ln2_ref[pl.ds(base, 16), :] for base in bases], axis=0)
    gate = jnp.dot(xsb, wg_ref[...], preferred_element_type=f32)
    up = jnp.dot(xsb, wu_ref[...], preferred_element_type=f32)
    act = (gate * jax.nn.sigmoid(gate) * up).astype(bf16)
    y = jnp.dot(act, wd_ref[...], preferred_element_type=f32)
    rid16 = lax.broadcasted_iota(jnp.int32, (16, D), 0)
    upds = []
    for c, (k, idx, base) in enumerate(zip((k1, k2), idxs, bases)):
        kv = k & jnp.int32(-65536)
        rsel = pltpu.bitcast(jnp.where(kv >= 0, kv, kv ^ jnp.int32(0x7FFF0000)), f32)
        gatew = jnp.concatenate([jax.nn.sigmoid(rsel)] * (D // 128), axis=1)
        upds.append(jnp.where(rid16 == idx - base, y[16 * c:16 * (c + 1)] * gatew, 0.0))
    for i in range(NO):
        out_copy(i).wait()
    for upd, base in zip(upds, bases):
        o_ref[pl.ds(base, 16), :] = (o_ref[pl.ds(base, 16), :].astype(f32) + upd).astype(bf16)

    def fix_copy(c):
        return pltpu.make_async_copy(o_ref.at[pl.ds(bases[c], 16)], out_hbm.at[pl.ds(bases[c], 16)], sems.at[c])

    fix_copy(0).start()

    @pl.when(bases[0] != bases[1])
    def _():
        fix_copy(1).start()
        fix_copy(1).wait()

    fix_copy(0).wait()


@jax.jit
def pallas_sequential_preLN__mha_block__moe_arch_mod__prompt_kernel(
    A_x: jax.Array,
    A_wqkv: jax.Array,
    A_wo: jax.Array,
    B_x: jax.Array,
    B_w_r: jax.Array,
    B_w_gate: jax.Array,
    B_w_up: jax.Array,
    B_w_down: jax.Array,
):
    del B_x
    any_spec = pl.BlockSpec(memory_space=pl.ANY)
    out = pl.pallas_call(
        _kernel,
        out_shape=jax.ShapeDtypeStruct((S, D), bf16),
        in_specs=[any_spec] * 7,
        out_specs=any_spec,
        scratch_shapes=[
            pltpu.VMEM((S, D), bf16),
            pltpu.VMEM((D, 3 * D), bf16),
            pltpu.VMEM((D, D), bf16),
            pltpu.VMEM((D // 2, D), jnp.int32),
            pltpu.VMEM((D,), bf16),
            pltpu.VMEM((D, F), bf16),
            pltpu.VMEM((D, F), bf16),
            pltpu.VMEM((F, D), bf16),
            pltpu.VMEM((2 * D, D), bf16),
            pltpu.VMEM((S, D), bf16),
            pltpu.VMEM((4, S // 2, 128), jnp.int32),
            pltpu.VMEM((NQ, 4, 128, TQ), bf16),
            pltpu.VMEM((H, DH // 2, S), jnp.int32),
            pltpu.VMEM((TOTAL + 2, DH, TQ), bf16),
            pltpu.VMEM((NCK, 8, D), f32),
            pltpu.VMEM((H, NCK, DH, 8, 128), f32),
            pltpu.VMEM((TOTAL, DH, TQ), f32),
            pltpu.VMEM((8 * CK, TQ), f32),
            pltpu.VMEM((8 * CK, TQ), f32),
            pltpu.VMEM((8 * CK, TQ), f32),
            pltpu.VMEM((8 * CK, TQ), f32),
            pltpu.VMEM((S, D), bf16),
            pltpu.VMEM((S, D), bf16),
            pltpu.SMEM((1,), jnp.int32),
            pltpu.SemaphoreType.DMA((6,)),
        ],
        compiler_params=pltpu.CompilerParams(vmem_limit_bytes=110 * 1024 * 1024),
    )(A_x.reshape(S, D), A_wqkv, A_wo, B_w_r, B_w_gate, B_w_up, B_w_down)
    return out.reshape(1, S, D)
```

```python
import jax
import jax.numpy as jnp
from jax import lax
import jax.experimental.pallas as pl
import jax.experimental.pallas.tpu as pltpu

S = 2048
D = 512
H = 32
DH = 16
F = 1792
EPS = 1e-5
QSCALE = (DH ** -0.5) * 1.4426950408889634

TA = 512
NA = S // TA
MQ = 128
TQ = 512
NQ = S // TQ
TOTAL = H * NQ
HPB = 8
CK = 128
NCK = S // CK
DLAG = NCK + 2
TC = 128
NC = S // TC
TO = 256
NO = S // TO

NEG_BIG = -3.0e38
LAGM = 3
PINT = (6, 6, 5, 4)
PSPLIT = 384
KB_PER_TILE = (0, 8, 16, 8)
GLAG = 2
PINC = 3
NTAIL = 2
NCOVER = 1

f32 = jnp.float32
bf16 = jnp.bfloat16
NN = (((1,), (0,)), ((), ()))
NT = (((1,), (1,)), ((), ()))


def _ln_stats(x):
    m = jnp.sum(x, axis=-1, keepdims=True) * (1.0 / D)
    v = jnp.maximum(jnp.sum(x * x, axis=-1, keepdims=True) * (1.0 / D) - m * m, 0.0)
    return m, lax.rsqrt(v + EPS)


def _layernorm(x):
    m = jnp.mean(x, axis=-1, keepdims=True)
    xc = x - m
    v = jnp.mean(xc * xc, axis=-1, keepdims=True)
    return xc * lax.rsqrt(v + EPS)


def _kernel(x_hbm, wqkv_hbm, wo_hbm, wr_hbm, wg_hbm, wu_hbm, wd_hbm, out_hbm,
            x_ref, wqkv_ref, wo_ref, wo32_ref, wr_ref, wg_ref, wu_ref, wd_ref, wt_ref, ln1_ref,
            k_ref, qt_ref, vt_ref, ot_ref, kf_ref, kb_ref, qf_ref, s0, s1, s2, s3,
            ln2_ref, o_ref, z_ref, sems):
    srefs = [s0, s1, s2, s3]

    def x_copy(i):
        return pltpu.make_async_copy(x_hbm.at[pl.ds(i * TA, TA)], x_ref.at[pl.ds(i * TA, TA)],
                                     sems.at[(0, 2, 2, 3)[i]])

    def wqkv_copy(part):
        cols = pl.ds(part * D, D)
        return pltpu.make_async_copy(wqkv_hbm.at[:, cols], wqkv_ref.at[:, cols], sems.at[(3, 1, 3)[part]])

    wo_copy = pltpu.make_async_copy(wo_hbm, wo_ref, sems.at[0])
    late_copies = [
        pltpu.make_async_copy(wr_hbm, wr_ref, sems.at[4]),
        pltpu.make_async_copy(wg_hbm, wg_ref, sems.at[4]),
        pltpu.make_async_copy(wu_hbm, wu_ref, sems.at[4]),
        pltpu.make_async_copy(wd_hbm, wd_ref, sems.at[4]),
    ]
    x_copy(0).start()
    wqkv_copy(1).start()
    for i in range(1, NA):
        x_copy(i).start()
    wqkv_copy(0).start()
    wqkv_copy(2).start()
    z_ref[0] = 0
    for sl in range(2 * NCK - DLAG, 2 * NCK):
        srefs[sl // 8][pl.ds((sl % 8) * CK, CK), :] = jnp.zeros((CK, TQ), f32)

    ln_deps = []

    def ln1(i, pin=False):
        rows = pl.ds(i * TA, TA)
        ln = _layernorm(x_ref[rows, :].astype(f32))
        ln1_ref[rows, :] = ln.astype(bf16)
        if pin:
            for u in range(TA // 8):
                row = ln[8 * u:8 * (u + 1)]
                ln_deps.append(jnp.minimum(jnp.minimum(row[:, 0:128], row[:, 128:256]),
                                           jnp.minimum(row[:, 256:384], row[:, 384:512])))

    jobs = []
    gates = []

    def paced(lhs, with_jobs, n_deps=0):
        if not with_jobs and n_deps == 0:
            return lhs
        n_tiles = (lhs.shape[0] // 16) * (lhs.shape[1] // 128)
        tile_no = 0
        w32 = pltpu.bitcast(lhs, jnp.int32)
        gate = gates[-GLAG] if len(gates) >= GLAG else None
        cols = []
        for kt in range(w32.shape[1] // 128):
            tiles = []
            for u in range(w32.shape[0] // 8):
                tile = w32[8 * u:8 * (u + 1), kt * 128:(kt + 1) * 128]
                lo = None
                src = {}
                tile_no += 1
                for _ in range(n_deps * tile_no // n_tiles - n_deps * (tile_no - 1) // n_tiles):
                    dep = ln_deps.pop(0)
                    lo = dep if lo is None else jnp.minimum(lo, dep)
                for _ in range(KB_PER_TILE[kt] if with_jobs else 0):
                    c, g, lane = jobs.pop(0)
                    if (c, g) not in src:
                        src[c, g] = jnp.where(gate < NEG_BIG, 0.0, kf_ref[c, :, g * 128:(g + 1) * 128])
                    kb = jnp.broadcast_to(src[c, g][:, lane:lane + 1], (8, 128))
                    col = g * 128 + lane
                    kb_ref[col // DH, c, col % DH] = kb
                    lo = kb if lo is None else jnp.minimum(lo, kb)
                tiles.append(tile if lo is None else jnp.where(lo < NEG_BIG, 0, tile))
            cols.append(jnp.concatenate(tiles, axis=0))
        return pltpu.bitcast(jnp.concatenate(cols, axis=1), bf16)

    def proj_k(lo, hi, pin_lo=None):
        for mb in range(lo, hi):
            r0 = mb * MQ
            rows = pl.ds(r0, MQ)
            n_deps = -(-len(ln_deps) // (hi - mb)) if (pin_lo is not None and mb >= pin_lo) else 0
            res = jnp.dot(paced(ln1_ref[rows, :], False, n_deps), wqkv_ref[:, D:2 * D],
                          preferred_element_type=f32)
            gates.append(res[0:8, 0:128])
            kk = res.astype(bf16)
            k32 = pltpu.bitcast(kk, jnp.int32)
            for g in range(4):
                k_ref[g, pl.ds(r0 // 2, MQ // 2), :] = k32[:, g * 128:(g + 1) * 128]
            if (r0 + MQ) % (2 * CK) == 0:
                c0 = 2 * (r0 // (2 * CK))
                kf_ref[pl.ds(c0, 2)] = kk[MQ - 16:MQ].astype(f32).reshape(2, 8, D)
                jobs.extend((c, g, lane) for c in (c0, c0 + 1) for g in range(4) for lane in range(128))

    def proj_qv(i):
        rows = pl.ds(i * TA, TA)
        for mb in range(2 * D // MQ):
            r0 = mb * MQ
            wt = paced(wt_ref[pl.ds(r0, MQ), :], True)
            res = lax.dot_general(wt, ln1_ref[rows, :], NT, preferred_element_type=f32)
            gates.append(res[0:8, 0:128])
            if r0 < D:
                qt = (res * QSCALE).astype(bf16)
                qf_ref[pl.ds(i * H + r0 // DH, MQ // DH)] = qt.astype(f32).reshape(MQ // DH, DH, TA)
                qt_ref[i, r0 // 128, pl.ds(r0 % 128, MQ), :] = qt
            else:
                vt_ref[pl.ds((r0 - D) // DH, MQ // DH), :, rows] = (
                    pltpu.bitcast(res.astype(bf16), jnp.int32).reshape(MQ // DH, DH // 2, TA))

    x_copy(0).wait()
    ln1(0)
    wqkv_copy(1).wait()
    proj_k(0, 3)
    x_copy(1).wait()
    x_copy(2).wait()
    proj_k(3, 4)
    ln1(1)
    ln1(2, pin=True)
    proj_k(4, 9, pin_lo=6)
    x_copy(3).wait()
    wqkv_copy(0).wait()
    wqkv_copy(2).wait()
    wo_copy.start()
    for c in late_copies:
        c.start()
    proj_k(9, 12)
    ln1(3)
    proj_k(12, 16)
    wt_ref[0:D, :] = wqkv_ref[:, 0:D].T
    wt_ref[D:2 * D, :] = wqkv_ref[:, 2 * D:3 * D].T
    for i in range(NA):
        proj_qv(i)
    assert not jobs
    wo_copy.wait()

    def qm_for(t0, hl):
        t = t0 + hl
        qb = t >> 5
        g = (t >> 3) & 3
        j = hl % 8
        parts = []
        if j > 0:
            parts.append(jnp.zeros((DH * j, TQ), bf16))
        parts.append(qt_ref[qb, g, j * DH:(j + 1) * DH, :])
        if j < 7:
            parts.append(jnp.zeros((DH * (7 - j), TQ), bf16))
        return jnp.concatenate(parts, axis=0), g

    def slot(n):
        sl = n % (2 * NCK)
        return srefs[sl // 8], (sl % 8) * CK

    def run(t0, n_hi, n_qk, ms, l, acc, extra=None):
        z = z_ref[0]
        ms = dict(ms)
        mx_hist = []
        mx = None
        mv = None
        for n in range(n_hi):
            if extra is not None:
                extra(n)
            if n < n_qk:
                hl, c = divmod(n, NCK)
                if c == 0:
                    qm, g = qm_for(t0, hl)
                sref, off = slot(n)
                nm = CK - 16 if c % 2 == 1 else CK
                t = t0 + hl
                kbs = [kb_ref[t & (H - 1), c, d] for d in range(DH)]
                cols = []
                for cc in range(TQ // 128):
                    parts = [None, None]
                    for d in range(DH):
                        term = kbs[d] * qf_ref[t, pl.ds(d, 1), cc * 128:(cc + 1) * 128]
                        parts[d % 2] = term if d < 2 else parts[d % 2] + term
                    cols.append(parts[0] + parts[1])
                sv = jnp.concatenate(cols, axis=1)
                sref2, off2 = slot(n | 1)
                sref2[pl.ds(off2 + CK - 16 + 8 * (c % 2), 8), :] = sv
                mv = sv if c == 0 else jnp.maximum(mv, sv)
                k32 = k_ref[g, pl.ds(c * CK // 2, nm // 2), :]
                tiles = [k32[8 * u:8 * (u + 1)] for u in range(nm // 16)]
                for cc, u in enumerate(PINT):
                    tiles[u] = jnp.where(mv[:, cc * 128:(cc + 1) * 128] < NEG_BIG, 0, tiles[u])
                kc = pltpu.bitcast(jnp.concatenate(tiles, axis=0), bf16)
                s = jnp.dot(kc, qm, preferred_element_type=f32)
                sref[pl.ds(off, nm), :] = s
                s3 = s.reshape(nm // 8, 8, TQ)
                for r in range(0, nm // 8, 2):
                    pm = jnp.maximum(s3[r], s3[r + 1])
                    mx = pm if (c == 0 and r == 0) else jnp.maximum(mx, pm)
                mx_hist.append(mx)
                if c == NCK - 1:
                    ms[hl] = jnp.broadcast_to(jnp.max(jnp.maximum(mx, mv), axis=0, keepdims=True), (8, TQ))
            hj, cj = divmod(n - DLAG, NCK)
            tj = t0 + hj
            h = tj & (H - 1)
            sref, off = slot(n - DLAG)
            drows = pl.ds(pl.multiple_of(off + z, CK), CK)
            m_eff = ms[hj]
            if n < n_qk and len(mx_hist) > LAGM:
                m_eff = jnp.maximum(m_eff, jnp.minimum(mx_hist[-1 - LAGM], NEG_BIG))
            p = jnp.exp2(sref[drows, :].reshape(CK // 8, 8, TQ) - m_eff[None])
            for r in range(CK // 8 - 2, -1, -2):
                pr = p[r + 1] + p[r]
                l = pr if (cj == 0 and r == CK // 8 - 2) else l + pr
            vt = pltpu.bitcast(vt_ref[h, :, pl.ds(cj * CK, CK)], bf16)
            p2 = p.reshape(CK, TQ)
            o = jnp.concatenate(
                [lax.dot_general(vt, p2[:, :PSPLIT].astype(bf16), NN, preferred_element_type=f32),
                 lax.dot_general(vt, p2[:, PSPLIT:], NN, preferred_element_type=f32)], axis=1)
            acc = o if cj == 0 else acc + o
            if cj == NCK - 1:
                lsum = jnp.sum(l, axis=0, keepdims=True)
                ot_ref[tj + 2] = (acc * (1.0 / lsum)).astype(bf16)
        return ms, l, acc

    def body(i, carry):
        ma, mb, l, acc = carry
        ms, l, acc = run(HPB * i, NCK * HPB, NCK * HPB, {-2: ma, -1: mb}, l, acc)
        return ms[HPB - 2], ms[HPB - 1], l, acc

    zeros8 = jnp.zeros((8, TQ), f32)
    ma, mb, l, acc = lax.fori_loop(0, TOTAL // HPB, body,
                                   (zeros8, zeros8, zeros8 + 1.0, jnp.zeros((DH, TQ), f32)))

    for c in late_copies:
        c.wait()

    def out_copy(i):
        return pltpu.make_async_copy(o_ref.at[pl.ds(i * TO, TO)], out_hbm.at[pl.ds(i * TO, TO)], sems.at[5])

    wr_row = wr_ref[...].reshape(1, D).astype(f32)
    wr_sum = jnp.sum(wr_row, axis=-1, keepdims=True)
    attn = {}
    deps = {}
    best = []
    int_min = jnp.iinfo(jnp.int32).min
    lane8 = lax.broadcasted_iota(jnp.int32, (8, 128), 1)
    row8 = lax.broadcasted_iota(jnp.int32, (8, 128), 0)

    def make_key(r, ids):
        bits = pltpu.bitcast(r.astype(bf16).astype(f32) + 0.0, jnp.int32)
        return jnp.where(bits >= 0, bits, bits ^ jnp.int32(0x7FFF0000)) | (S - 1 - ids)

    def insert(key):
        if not best:
            best.extend([key, jnp.full((8, 128), int_min, jnp.int32)])
        else:
            lo = jnp.minimum(best[0], key)
            best[0] = jnp.maximum(best[0], key)
            best[1] = jnp.maximum(best[1], lo)

    def all_max(v):
        return jnp.broadcast_to(jnp.max(jnp.max(v, axis=0, keepdims=True), axis=1, keepdims=True), (1, 128))

    def c_proj(i):
        qb, part = divmod(i, TQ // TC)
        o_nat = ot_ref[pl.ds(2 + qb * H, H), :, pl.ds(part * TC, TC)].reshape(D, TC).T
        if i - PINC in deps:
            zero = jnp.where(jnp.concatenate(deps.pop(i - PINC), axis=0) < NEG_BIG, -1, 0)
            head = pltpu.bitcast(pltpu.bitcast(o_nat[:, 0:128], jnp.int32) | zero, bf16)
            o_nat = jnp.concatenate([head, o_nat[:, 128:]], axis=1)
        if i == 1:
            wo32_ref[...] = pltpu.bitcast(wo_ref[...], jnp.int32)
        wo = wo_ref[...] if i == 0 else pltpu.bitcast(wo32_ref[...], bf16)
        attn[i] = jnp.dot(o_nat, wo, preferred_element_type=f32)

    def c_norm(i):
        rows = pl.ds(i * TC, TC)
        hh = x_ref[rows, :].astype(f32) + attn.pop(i)
        m, rstd = _ln_stats(hh)
        ln2 = (hh - m) * rstd
        ln2_ref[rows, :] = ln2.astype(bf16)
        o_ref[rows, :] = (hh + ln2).astype(bf16)
        if ((i + 1) * TC) % TO == 0:
            out_copy((i * TC) // TO).start()
        r = jnp.broadcast_to((jnp.sum(hh * wr_row, axis=-1, keepdims=True) - m * wr_sum) * rstd, (TC, 128))
        if i < NC - NTAIL:
            rc = r[0:8]
            for u in range(1, TC // 8):
                rc = jnp.where(lane8 == u, r[8 * u:8 * (u + 1)], rc)
                if u % 2 == 1:
                    deps.setdefault(i, []).append(rc)
            insert(jnp.where(lane8 < TC // 8, make_key(rc, i * TC + 8 * lane8 + row8), int_min))
            if i == NC - NTAIL - 1:
                k1 = all_max(best[0])
                k2 = all_max(jnp.where(best[0] == k1, best[1], best[0]))
                best[0] = jnp.where(row8 == 0, k1, int_min)
                best[1] = jnp.where(row8 == 0, k2, int_min)
        else:
            for u in range(TC // 8):
                insert(make_key(r[8 * u:8 * (u + 1)], i * TC + 8 * u + row8))

    n_early = (NQ - 1) * (TQ // TC) - NCOVER

    def c_step(i):
        if i < NC:
            c_proj(i)
        if i >= 1:
            c_norm(i - 1)

    def extra(n):
        for i in range(n * n_early // DLAG, (n + 1) * n_early // DLAG):
            c_step(i)

    run(TOTAL, DLAG, 0, {-2: ma, -1: mb}, l, acc, extra=extra)
    for i in range(n_early, NC + 1):
        c_step(i)

    k1 = jnp.max(best[0], axis=0, keepdims=True)
    k2 = jnp.max(jnp.where(best[0] == k1, best[1], best[0]), axis=0, keepdims=True)
    idxs = [S - 1 - (k[0, 0] & (S - 1)) for k in (k1, k2)]
    bases = [pl.multiple_of((idx >> 4) << 4, 16) for idx in idxs]

    xsb = jnp.concatenate([ln2_ref[pl.ds(base, 16), :] for base in bases], axis=0)
    gate = jnp.dot(xsb, wg_ref[...], preferred_element_type=f32)
    up = jnp.dot(xsb, wu_ref[...], preferred_element_type=f32)
    act = (gate * jax.nn.sigmoid(gate) * up).astype(bf16)
    y = jnp.dot(act, wd_ref[...], preferred_element_type=f32)
    rid16 = lax.broadcasted_iota(jnp.int32, (16, D), 0)
    upds = []
    for c, (k, idx, base) in enumerate(zip((k1, k2), idxs, bases)):
        kv = k & jnp.int32(-65536)
        rsel = pltpu.bitcast(jnp.where(kv >= 0, kv, kv ^ jnp.int32(0x7FFF0000)), f32)
        gatew = jnp.concatenate([jax.nn.sigmoid(rsel)] * (D // 128), axis=1)
        upds.append(jnp.where(rid16 == idx - base, y[16 * c:16 * (c + 1)] * gatew, 0.0))
    for i in range(NO):
        out_copy(i).wait()
    for upd, base in zip(upds, bases):
        o_ref[pl.ds(base, 16), :] = (o_ref[pl.ds(base, 16), :].astype(f32) + upd).astype(bf16)

    def fix_copy(c):
        return pltpu.make_async_copy(o_ref.at[pl.ds(bases[c], 16)], out_hbm.at[pl.ds(bases[c], 16)], sems.at[c])

    fix_copy(0).start()

    @pl.when(bases[0] != bases[1])
    def _():
        fix_copy(1).start()
        fix_copy(1).wait()

    fix_copy(0).wait()


@jax.jit
def pallas_sequential_preLN__mha_block__moe_arch_mod__prompt_kernel(
    A_x: jax.Array,
    A_wqkv: jax.Array,
    A_wo: jax.Array,
    B_x: jax.Array,
    B_w_r: jax.Array,
    B_w_gate: jax.Array,
    B_w_up: jax.Array,
    B_w_down: jax.Array,
):
    del B_x
    any_spec = pl.BlockSpec(memory_space=pl.ANY)
    out = pl.pallas_call(
        _kernel,
        out_shape=jax.ShapeDtypeStruct((S, D), bf16),
        in_specs=[any_spec] * 7,
        out_specs=any_spec,
        scratch_shapes=[
            pltpu.VMEM((S, D), bf16),
            pltpu.VMEM((D, 3 * D), bf16),
            pltpu.VMEM((D, D), bf16),
            pltpu.VMEM((D // 2, D), jnp.int32),
            pltpu.VMEM((D,), bf16),
            pltpu.VMEM((D, F), bf16),
            pltpu.VMEM((D, F), bf16),
            pltpu.VMEM((F, D), bf16),
            pltpu.VMEM((2 * D, D), bf16),
            pltpu.VMEM((S, D), bf16),
            pltpu.VMEM((4, S // 2, 128), jnp.int32),
            pltpu.VMEM((NQ, 4, 128, TQ), bf16),
            pltpu.VMEM((H, DH // 2, S), jnp.int32),
            pltpu.VMEM((TOTAL + 2, DH, TQ), bf16),
            pltpu.VMEM((NCK, 8, D), f32),
            pltpu.VMEM((H, NCK, DH, 8, 128), f32),
            pltpu.VMEM((TOTAL, DH, TQ), f32),
            pltpu.VMEM((8 * CK, TQ), f32),
            pltpu.VMEM((8 * CK, TQ), f32),
            pltpu.VMEM((8 * CK, TQ), f32),
            pltpu.VMEM((8 * CK, TQ), f32),
            pltpu.VMEM((S, D), bf16),
            pltpu.VMEM((S, D), bf16),
            pltpu.SMEM((1,), jnp.int32),
            pltpu.SemaphoreType.DMA((6,)),
        ],
        compiler_params=pltpu.CompilerParams(vmem_limit_bytes=110 * 1024 * 1024),
    )(A_x.reshape(S, D), A_wqkv, A_wo, B_w_r, B_w_gate, B_w_up, B_w_down)
    return out.reshape(1, S, D)
```

```python
import jax
import jax.numpy as jnp
from jax import lax
import jax.experimental.pallas as pl
import jax.experimental.pallas.tpu as pltpu

S = 2048
D = 512
H = 32
DH = 16
F = 1792
EPS = 1e-5
QSCALE = (DH ** -0.5) * 1.4426950408889634

TA = 512
NA = S // TA
MQ = 128
TQ = 512
NQ = S // TQ
TOTAL = H * NQ
HPB = 8
CK = 128
NCK = S // CK
DLAG = NCK + 2
TC = 128
NC = S // TC
TO = 256
NO = S // TO

NEG_BIG = -3.0e38
LAGM = 3
PINT = (6, 6, 5, 4)
PSPLIT = 384
KB_PER_TILE = (0, 8, 16, 8)
GLAG = 2
PINC = 3
NTAIL = 2
NCOVER = 1

f32 = jnp.float32
bf16 = jnp.bfloat16
NN = (((1,), (0,)), ((), ()))
NT = (((1,), (1,)), ((), ()))


def _ln_stats(x):
    m = jnp.sum(x, axis=-1, keepdims=True) * (1.0 / D)
    v = jnp.maximum(jnp.sum(x * x, axis=-1, keepdims=True) * (1.0 / D) - m * m, 0.0)
    return m, lax.rsqrt(v + EPS)


def _layernorm(x):
    m = jnp.mean(x, axis=-1, keepdims=True)
    xc = x - m
    v = jnp.mean(xc * xc, axis=-1, keepdims=True)
    return xc * lax.rsqrt(v + EPS)


def _kernel(x_hbm, wqkv_hbm, wo_hbm, wr_hbm, wg_hbm, wu_hbm, wd_hbm, out_hbm,
            x_ref, wq_ref, wk_ref, wv_ref, wo_ref, wo32_ref, wr_ref, wg_ref, wu_ref, wd_ref, wt_ref, ln1_ref,
            k_ref, qt_ref, vt_ref, ot_ref, kf_ref, kb_ref, qf_ref, s0, s1, s2, s3,
            ln2_ref, o_ref, z_ref, sems):
    srefs = [s0, s1, s2, s3]

    def x_copy(i):
        return pltpu.make_async_copy(x_hbm.at[pl.ds(i * TA, TA)], x_ref.at[pl.ds(i * TA, TA)],
                                     sems.at[(0, 2, 2, 3)[i]])

    def wqkv_copy(part):
        return pltpu.make_async_copy(wqkv_hbm.at[:, pl.ds(part * D, D)], (wq_ref, wk_ref, wv_ref)[part],
                                     sems.at[(3, 1, 3)[part]])

    wo_copy = pltpu.make_async_copy(wo_hbm, wo_ref, sems.at[0])
    late_copies = [
        pltpu.make_async_copy(wr_hbm, wr_ref, sems.at[4]),
        pltpu.make_async_copy(wg_hbm, wg_ref, sems.at[4]),
        pltpu.make_async_copy(wu_hbm, wu_ref, sems.at[4]),
        pltpu.make_async_copy(wd_hbm, wd_ref, sems.at[4]),
    ]
    x_copy(0).start()
    wqkv_copy(1).start()
    for i in range(1, NA):
        x_copy(i).start()
    wqkv_copy(0).start()
    wqkv_copy(2).start()
    z_ref[0] = 0
    for sl in range(2 * NCK - DLAG, 2 * NCK):
        srefs[sl // 8][pl.ds((sl % 8) * CK, CK), :] = jnp.zeros((CK, TQ), f32)

    ln_deps = []

    def ln1(i, pin=False):
        rows = pl.ds(i * TA, TA)
        ln = _layernorm(x_ref[rows, :].astype(f32))
        ln1_ref[rows, :] = ln.astype(bf16)
        if pin:
            for u in range(TA // 8):
                row = ln[8 * u:8 * (u + 1)]
                ln_deps.append(jnp.minimum(jnp.minimum(row[:, 0:128], row[:, 128:256]),
                                           jnp.minimum(row[:, 256:384], row[:, 384:512])))

    jobs = []
    gates = []

    def paced(lhs, with_jobs, n_deps=0):
        if not with_jobs and n_deps == 0:
            return lhs
        n_tiles = (lhs.shape[0] // 16) * (lhs.shape[1] // 128)
        tile_no = 0
        w32 = pltpu.bitcast(lhs, jnp.int32)
        gate = gates[-GLAG] if len(gates) >= GLAG else None
        cols = []
        for kt in range(w32.shape[1] // 128):
            tiles = []
            for u in range(w32.shape[0] // 8):
                tile = w32[8 * u:8 * (u + 1), kt * 128:(kt + 1) * 128]
                lo = None
                src = {}
                tile_no += 1
                for _ in range(n_deps * tile_no // n_tiles - n_deps * (tile_no - 1) // n_tiles):
                    dep = ln_deps.pop(0)
                    lo = dep if lo is None else jnp.minimum(lo, dep)
                for _ in range(KB_PER_TILE[kt] if with_jobs else 0):
                    c, g, lane = jobs.pop(0)
                    if (c, g) not in src:
                        src[c, g] = jnp.where(gate < NEG_BIG, 0.0, kf_ref[c, :, g * 128:(g + 1) * 128])
                    kb = jnp.broadcast_to(src[c, g][:, lane:lane + 1], (8, 128))
                    col = g * 128 + lane
                    kb_ref[col // DH, c, col % DH] = kb
                    lo = kb if lo is None else jnp.minimum(lo, kb)
                tiles.append(tile if lo is None else jnp.where(lo < NEG_BIG, 0, tile))
            cols.append(jnp.concatenate(tiles, axis=0))
        return pltpu.bitcast(jnp.concatenate(cols, axis=1), bf16)

    def proj_k(lo, hi, pin_lo=None):
        for mb in range(lo, hi):
            r0 = mb * MQ
            rows = pl.ds(r0, MQ)
            n_deps = -(-len(ln_deps) // (hi - mb)) if (pin_lo is not None and mb >= pin_lo) else 0
            res = jnp.dot(paced(ln1_ref[rows, :], False, n_deps), wk_ref[...], preferred_element_type=f32)
            gates.append(res[0:8, 0:128])
            kk = res.astype(bf16)
            k32 = pltpu.bitcast(kk, jnp.int32)
            for g in range(4):
                k_ref[g, pl.ds(r0 // 2, MQ // 2), :] = k32[:, g * 128:(g + 1) * 128]
            if (r0 + MQ) % (2 * CK) == 0:
                c0 = 2 * (r0 // (2 * CK))
                kf_ref[pl.ds(c0, 2)] = kk[MQ - 16:MQ].astype(f32).reshape(2, 8, D)
                jobs.extend((c, g, lane) for c in (c0, c0 + 1) for g in range(4) for lane in range(128))

    def proj_qv(i):
        rows = pl.ds(i * TA, TA)
        for mb in range(2 * D // MQ):
            r0 = mb * MQ
            wt = paced(wt_ref[pl.ds(r0, MQ), :], True)
            res = lax.dot_general(wt, ln1_ref[rows, :], NT, preferred_element_type=f32)
            gates.append(res[0:8, 0:128])
            if r0 < D:
                qt = (res * QSCALE).astype(bf16)
                qf_ref[pl.ds(i * H + r0 // DH, MQ // DH)] = qt.astype(f32).reshape(MQ // DH, DH, TA)
                qt_ref[i, r0 // 128, pl.ds(r0 % 128, MQ), :] = qt
            else:
                vt_ref[pl.ds((r0 - D) // DH, MQ // DH), :, rows] = (
                    pltpu.bitcast(res.astype(bf16), jnp.int32).reshape(MQ // DH, DH // 2, TA))

    x_copy(0).wait()
    ln1(0)
    wqkv_copy(1).wait()
    proj_k(0, 3)
    x_copy(1).wait()
    x_copy(2).wait()
    proj_k(3, 4)
    ln1(1)
    ln1(2, pin=True)
    proj_k(4, 9, pin_lo=6)
    x_copy(3).wait()
    wqkv_copy(0).wait()
    wqkv_copy(2).wait()
    wo_copy.start()
    for c in late_copies:
        c.start()
    proj_k(9, 12)
    ln1(3)
    proj_k(12, 16)
    wt_ref[0:D, :] = wq_ref[...].T
    wt_ref[D:2 * D, :] = wv_ref[...].T
    for i in range(NA):
        proj_qv(i)
    assert not jobs
    wo_copy.wait()

    def qm_for(t0, hl):
        t = t0 + hl
        qb = t >> 5
        g = (t >> 3) & 3
        j = hl % 8
        parts = []
        if j > 0:
            parts.append(jnp.zeros((DH * j, TQ), bf16))
        parts.append(qt_ref[qb, g, j * DH:(j + 1) * DH, :])
        if j < 7:
            parts.append(jnp.zeros((DH * (7 - j), TQ), bf16))
        return jnp.concatenate(parts, axis=0), g

    def slot(n):
        sl = n % (2 * NCK)
        return srefs[sl // 8], (sl % 8) * CK

    def run(t0, n_hi, n_qk, ms, l, acc, extra=None):
        z = z_ref[0]
        ms = dict(ms)
        mx_hist = []
        mx = None
        mv = None
        for n in range(n_hi):
            if extra is not None:
                extra(n)
            if n < n_qk:
                hl, c = divmod(n, NCK)
                if c == 0:
                    qm, g = qm_for(t0, hl)
                sref, off = slot(n)
                nm = CK - 16 if c % 2 == 1 else CK
                t = t0 + hl
                kbs = [kb_ref[t & (H - 1), c, d] for d in range(DH)]
                cols = []
                for cc in range(TQ // 128):
                    parts = [None, None]
                    for d in range(DH):
                        term = kbs[d] * qf_ref[t, pl.ds(d, 1), cc * 128:(cc + 1) * 128]
                        parts[d % 2] = term if d < 2 else parts[d % 2] + term
                    cols.append(parts[0] + parts[1])
                sv = jnp.concatenate(cols, axis=1)
                sref2, off2 = slot(n | 1)
                sref2[pl.ds(off2 + CK - 16 + 8 * (c % 2), 8), :] = sv
                mv = sv if c == 0 else jnp.maximum(mv, sv)
                k32 = k_ref[g, pl.ds(c * CK // 2, nm // 2), :]
                tiles = [k32[8 * u:8 * (u + 1)] for u in range(nm // 16)]
                for cc, u in enumerate(PINT):
                    tiles[u] = jnp.where(mv[:, cc * 128:(cc + 1) * 128] < NEG_BIG, 0, tiles[u])
                kc = pltpu.bitcast(jnp.concatenate(tiles, axis=0), bf16)
                s = jnp.dot(kc, qm, preferred_element_type=f32)
                sref[pl.ds(off, nm), :] = s
                s3 = s.reshape(nm // 8, 8, TQ)
                for r in range(0, nm // 8, 2):
                    pm = jnp.maximum(s3[r], s3[r + 1])
                    mx = pm if (c == 0 and r == 0) else jnp.maximum(mx, pm)
                mx_hist.append(mx)
                if c == NCK - 1:
                    ms[hl] = jnp.broadcast_to(jnp.max(jnp.maximum(mx, mv), axis=0, keepdims=True), (8, TQ))
            hj, cj = divmod(n - DLAG, NCK)
            tj = t0 + hj
            h = tj & (H - 1)
            sref, off = slot(n - DLAG)
            drows = pl.ds(pl.multiple_of(off + z, CK), CK)
            m_eff = ms[hj]
            if n < n_qk and len(mx_hist) > LAGM:
                m_eff = jnp.maximum(m_eff, jnp.minimum(mx_hist[-1 - LAGM], NEG_BIG))
            p = jnp.exp2(sref[drows, :].reshape(CK // 8, 8, TQ) - m_eff[None])
            for r in range(CK // 8 - 2, -1, -2):
                pr = p[r + 1] + p[r]
                l = pr if (cj == 0 and r == CK // 8 - 2) else l + pr
            vt = pltpu.bitcast(vt_ref[h, :, pl.ds(cj * CK, CK)], bf16)
            p2 = p.reshape(CK, TQ)
            o = jnp.concatenate(
                [lax.dot_general(vt, p2[:, :PSPLIT].astype(bf16), NN, preferred_element_type=f32),
                 lax.dot_general(vt, p2[:, PSPLIT:], NN, preferred_element_type=f32)], axis=1)
            acc = o if cj == 0 else acc + o
            if cj == NCK - 1:
                lsum = jnp.sum(l, axis=0, keepdims=True)
                ot_ref[tj + 2] = (acc * (1.0 / lsum)).astype(bf16)
        return ms, l, acc

    def body(i, carry):
        ma, mb, l, acc = carry
        ms, l, acc = run(HPB * i, NCK * HPB, NCK * HPB, {-2: ma, -1: mb}, l, acc)
        return ms[HPB - 2], ms[HPB - 1], l, acc

    zeros8 = jnp.zeros((8, TQ), f32)
    ma, mb, l, acc = lax.fori_loop(0, TOTAL // HPB, body,
                                   (zeros8, zeros8, zeros8 + 1.0, jnp.zeros((DH, TQ), f32)))

    for c in late_copies:
        c.wait()

    def out_copy(i):
        return pltpu.make_async_copy(o_ref.at[pl.ds(i * TO, TO)], out_hbm.at[pl.ds(i * TO, TO)], sems.at[5])

    wr_row = wr_ref[...].reshape(1, D).astype(f32)
    wr_sum = jnp.sum(wr_row, axis=-1, keepdims=True)
    attn = {}
    deps = {}
    best = []
    int_min = jnp.iinfo(jnp.int32).min
    lane8 = lax.broadcasted_iota(jnp.int32, (8, 128), 1)
    row8 = lax.broadcasted_iota(jnp.int32, (8, 128), 0)

    def make_key(r, ids):
        bits = pltpu.bitcast(r.astype(bf16).astype(f32) + 0.0, jnp.int32)
        return jnp.where(bits >= 0, bits, bits ^ jnp.int32(0x7FFF0000)) | (S - 1 - ids)

    def insert(key):
        if not best:
            best.extend([key, jnp.full((8, 128), int_min, jnp.int32)])
        else:
            lo = jnp.minimum(best[0], key)
            best[0] = jnp.maximum(best[0], key)
            best[1] = jnp.maximum(best[1], lo)

    def all_max(v):
        return jnp.broadcast_to(jnp.max(jnp.max(v, axis=0, keepdims=True), axis=1, keepdims=True), (1, 128))

    def c_proj(i):
        qb, part = divmod(i, TQ // TC)
        o_nat = ot_ref[pl.ds(2 + qb * H, H), :, pl.ds(part * TC, TC)].reshape(D, TC).T
        if i - PINC in deps:
            zero = jnp.where(jnp.concatenate(deps.pop(i - PINC), axis=0) < NEG_BIG, -1, 0)
            head = pltpu.bitcast(pltpu.bitcast(o_nat[:, 0:128], jnp.int32) | zero, bf16)
            o_nat = jnp.concatenate([head, o_nat[:, 128:]], axis=1)
        if i == 1:
            wo32_ref[...] = pltpu.bitcast(wo_ref[...], jnp.int32)
        wo = wo_ref[...] if i == 0 else pltpu.bitcast(wo32_ref[...], bf16)
        attn[i] = jnp.dot(o_nat, wo, preferred_element_type=f32)

    def c_norm(i):
        rows = pl.ds(i * TC, TC)
        hh = x_ref[rows, :].astype(f32) + attn.pop(i)
        m, rstd = _ln_stats(hh)
        ln2 = (hh - m) * rstd
        ln2_ref[rows, :] = ln2.astype(bf16)
        o_ref[rows, :] = (hh + ln2).astype(bf16)
        if ((i + 1) * TC) % TO == 0:
            out_copy((i * TC) // TO).start()
        r = jnp.broadcast_to((jnp.sum(hh * wr_row, axis=-1, keepdims=True) - m * wr_sum) * rstd, (TC, 128))
        if i < NC - NTAIL:
            rc = r[0:8]
            for u in range(1, TC // 8):
                rc = jnp.where(lane8 == u, r[8 * u:8 * (u + 1)], rc)
                if u % 2 == 1:
                    deps.setdefault(i, []).append(rc)
            insert(jnp.where(lane8 < TC // 8, make_key(rc, i * TC + 8 * lane8 + row8), int_min))
            if i == NC - NTAIL - 1:
                k1 = all_max(best[0])
                k2 = all_max(jnp.where(best[0] == k1, best[1], best[0]))
                best[0] = jnp.where(row8 == 0, k1, int_min)
                best[1] = jnp.where(row8 == 0, k2, int_min)
        else:
            for u in range(TC // 8):
                insert(make_key(r[8 * u:8 * (u + 1)], i * TC + 8 * u + row8))

    n_early = (NQ - 1) * (TQ // TC) - NCOVER

    def c_step(i):
        if i < NC:
            c_proj(i)
        if i >= 1:
            c_norm(i - 1)

    def extra(n):
        for i in range(n * n_early // DLAG, (n + 1) * n_early // DLAG):
            c_step(i)

    run(TOTAL, DLAG, 0, {-2: ma, -1: mb}, l, acc, extra=extra)
    for i in range(n_early, NC + 1):
        c_step(i)

    k1 = jnp.max(best[0], axis=0, keepdims=True)
    k2 = jnp.max(jnp.where(best[0] == k1, best[1], best[0]), axis=0, keepdims=True)
    idxs = [S - 1 - (k[0, 0] & (S - 1)) for k in (k1, k2)]
    bases = [pl.multiple_of((idx >> 4) << 4, 16) for idx in idxs]

    xsb = jnp.concatenate([ln2_ref[pl.ds(base, 16), :] for base in bases], axis=0)
    gate = jnp.dot(xsb, wg_ref[...], preferred_element_type=f32)
    up = jnp.dot(xsb, wu_ref[...], preferred_element_type=f32)
    act = (gate * jax.nn.sigmoid(gate) * up).astype(bf16)
    y = jnp.dot(act, wd_ref[...], preferred_element_type=f32)
    rid16 = lax.broadcasted_iota(jnp.int32, (16, D), 0)
    upds = []
    for c, (k, idx, base) in enumerate(zip((k1, k2), idxs, bases)):
        kv = k & jnp.int32(-65536)
        rsel = pltpu.bitcast(jnp.where(kv >= 0, kv, kv ^ jnp.int32(0x7FFF0000)), f32)
        gatew = jnp.concatenate([jax.nn.sigmoid(rsel)] * (D // 128), axis=1)
        upds.append(jnp.where(rid16 == idx - base, y[16 * c:16 * (c + 1)] * gatew, 0.0))
    for i in range(NO):
        out_copy(i).wait()
    for upd, base in zip(upds, bases):
        o_ref[pl.ds(base, 16), :] = (o_ref[pl.ds(base, 16), :].astype(f32) + upd).astype(bf16)

    def fix_copy(c):
        return pltpu.make_async_copy(o_ref.at[pl.ds(bases[c], 16)], out_hbm.at[pl.ds(bases[c], 16)], sems.at[c])

    fix_copy(0).start()

    @pl.when(bases[0] != bases[1])
    def _():
        fix_copy(1).start()
        fix_copy(1).wait()

    fix_copy(0).wait()


@jax.jit
def pallas_sequential_preLN__mha_block__moe_arch_mod__prompt_kernel(
    A_x: jax.Array,
    A_wqkv: jax.Array,
    A_wo: jax.Array,
    B_x: jax.Array,
    B_w_r: jax.Array,
    B_w_gate: jax.Array,
    B_w_up: jax.Array,
    B_w_down: jax.Array,
):
    del B_x
    any_spec = pl.BlockSpec(memory_space=pl.ANY)
    out = pl.pallas_call(
        _kernel,
        out_shape=jax.ShapeDtypeStruct((S, D), bf16),
        in_specs=[any_spec] * 7,
        out_specs=any_spec,
        scratch_shapes=[
            pltpu.VMEM((S, D), bf16),
            pltpu.VMEM((D, D), bf16),
            pltpu.VMEM((D, D), bf16),
            pltpu.VMEM((D, D), bf16),
            pltpu.VMEM((D, D), bf16),
            pltpu.VMEM((D // 2, D), jnp.int32),
            pltpu.VMEM((D,), bf16),
            pltpu.VMEM((D, F), bf16),
            pltpu.VMEM((D, F), bf16),
            pltpu.VMEM((F, D), bf16),
            pltpu.VMEM((2 * D, D), bf16),
            pltpu.VMEM((S, D), bf16),
            pltpu.VMEM((4, S // 2, 128), jnp.int32),
            pltpu.VMEM((NQ, 4, 128, TQ), bf16),
            pltpu.VMEM((H, DH // 2, S), jnp.int32),
            pltpu.VMEM((TOTAL + 2, DH, TQ), bf16),
            pltpu.VMEM((NCK, 8, D), f32),
            pltpu.VMEM((H, NCK, DH, 8, 128), f32),
            pltpu.VMEM((TOTAL, DH, TQ), f32),
            pltpu.VMEM((8 * CK, TQ), f32),
            pltpu.VMEM((8 * CK, TQ), f32),
            pltpu.VMEM((8 * CK, TQ), f32),
            pltpu.VMEM((8 * CK, TQ), f32),
            pltpu.VMEM((S, D), bf16),
            pltpu.VMEM((S, D), bf16),
            pltpu.SMEM((1,), jnp.int32),
            pltpu.SemaphoreType.DMA((6,)),
        ],
        compiler_params=pltpu.CompilerParams(vmem_limit_bytes=110 * 1024 * 1024),
    )(A_x.reshape(S, D), A_wqkv, A_wo, B_w_r, B_w_gate, B_w_up, B_w_down)
    return out.reshape(1, S, D)
```

```python
import jax
import jax.numpy as jnp
from jax import lax
import jax.experimental.pallas as pl
import jax.experimental.pallas.tpu as pltpu

S = 2048
D = 512
H = 32
DH = 16
F = 1792
EPS = 1e-5
QSCALE = (DH ** -0.5) * 1.4426950408889634

TA = 512
NA = S // TA
MQ = 128
TQ = 512
NQ = S // TQ
TOTAL = H * NQ
HPB = 8
CK = 128
NCK = S // CK
DLAG = NCK + 2
TC = 128
NC = S // TC
TO = 256
NO = S // TO

NEG_BIG = -3.0e38
LAGM = 3
PINT = (4, 5, 6, 6)
PSPLIT = 384
KB_PER_TILE = (0, 8, 16, 8)
GLAG = 2
PINC = 3
NTAIL = 2
NCOVER = 1

f32 = jnp.float32
bf16 = jnp.bfloat16
NN = (((1,), (0,)), ((), ()))
NT = (((1,), (1,)), ((), ()))


def _ln_stats(x):
    m = jnp.sum(x, axis=-1, keepdims=True) * (1.0 / D)
    v = jnp.maximum(jnp.sum(x * x, axis=-1, keepdims=True) * (1.0 / D) - m * m, 0.0)
    return m, lax.rsqrt(v + EPS)


def _layernorm(x):
    m = jnp.mean(x, axis=-1, keepdims=True)
    xc = x - m
    v = jnp.mean(xc * xc, axis=-1, keepdims=True)
    return xc * lax.rsqrt(v + EPS)


def _kernel(x_hbm, wqkv_hbm, wo_hbm, wr_hbm, wg_hbm, wu_hbm, wd_hbm, out_hbm,
            x_ref, wq_ref, wk_ref, wv_ref, wo_ref, wo32_ref, wr_ref, wg_ref, wu_ref, wd_ref, wt_ref, ln1_ref,
            k_ref, qt_ref, vt_ref, ot_ref, kf_ref, kb_ref, qf_ref, s0, s1, s2, s3,
            ln2_ref, o_ref, z_ref, sems):
    srefs = [s0, s1, s2, s3]

    def x_copy(i):
        return pltpu.make_async_copy(x_hbm.at[pl.ds(i * TA, TA)], x_ref.at[pl.ds(i * TA, TA)],
                                     sems.at[(0, 2, 2, 3)[i]])

    def wqkv_copy(part):
        return pltpu.make_async_copy(wqkv_hbm.at[:, pl.ds(part * D, D)], (wq_ref, wk_ref, wv_ref)[part],
                                     sems.at[(3, 1, 3)[part]])

    wo_copy = pltpu.make_async_copy(wo_hbm, wo_ref, sems.at[0])
    late_copies = [
        pltpu.make_async_copy(wr_hbm, wr_ref, sems.at[4]),
        pltpu.make_async_copy(wg_hbm, wg_ref, sems.at[4]),
        pltpu.make_async_copy(wu_hbm, wu_ref, sems.at[4]),
        pltpu.make_async_copy(wd_hbm, wd_ref, sems.at[4]),
    ]
    x_copy(0).start()
    wqkv_copy(1).start()
    for i in range(1, NA):
        x_copy(i).start()
    wqkv_copy(0).start()
    wqkv_copy(2).start()
    z_ref[0] = 0
    for sl in range(2 * NCK - DLAG, 2 * NCK):
        srefs[sl // 8][pl.ds((sl % 8) * CK, CK), :] = jnp.zeros((CK, TQ), f32)

    ln_deps = []

    def ln1(i, pin=False):
        rows = pl.ds(i * TA, TA)
        ln = _layernorm(x_ref[rows, :].astype(f32))
        ln1_ref[rows, :] = ln.astype(bf16)
        if pin:
            for u in range(TA // 8):
                row = ln[8 * u:8 * (u + 1)]
                ln_deps.append(jnp.minimum(jnp.minimum(row[:, 0:128], row[:, 128:256]),
                                           jnp.minimum(row[:, 256:384], row[:, 384:512])))

    jobs = []
    gates = []

    def paced(lhs, with_jobs, n_deps=0):
        if not with_jobs and n_deps == 0:
            return lhs
        n_tiles = (lhs.shape[0] // 16) * (lhs.shape[1] // 128)
        tile_no = 0
        w32 = pltpu.bitcast(lhs, jnp.int32)
        gate = gates[-GLAG] if len(gates) >= GLAG else None
        cols = []
        for kt in range(w32.shape[1] // 128):
            tiles = []
            for u in range(w32.shape[0] // 8):
                tile = w32[8 * u:8 * (u + 1), kt * 128:(kt + 1) * 128]
                lo = None
                src = {}
                tile_no += 1
                for _ in range(n_deps * tile_no // n_tiles - n_deps * (tile_no - 1) // n_tiles):
                    dep = ln_deps.pop(0)
                    lo = dep if lo is None else jnp.minimum(lo, dep)
                for _ in range(KB_PER_TILE[kt] if with_jobs else 0):
                    c, g, lane = jobs.pop(0)
                    if (c, g) not in src:
                        src[c, g] = jnp.where(gate < NEG_BIG, 0.0, kf_ref[c, :, g * 128:(g + 1) * 128])
                    kb = jnp.broadcast_to(src[c, g][:, lane:lane + 1], (8, 128))
                    col = g * 128 + lane
                    kb_ref[col // DH, c, col % DH] = kb
                    lo = kb if lo is None else jnp.minimum(lo, kb)
                tiles.append(tile if lo is None else jnp.where(lo < NEG_BIG, 0, tile))
            cols.append(jnp.concatenate(tiles, axis=0))
        return pltpu.bitcast(jnp.concatenate(cols, axis=1), bf16)

    def proj_k(lo, hi, pin_lo=None):
        for mb in range(lo, hi):
            r0 = mb * MQ
            rows = pl.ds(r0, MQ)
            n_deps = -(-len(ln_deps) // (hi - mb)) if (pin_lo is not None and mb >= pin_lo) else 0
            res = jnp.dot(paced(ln1_ref[rows, :], False, n_deps), wk_ref[...], preferred_element_type=f32)
            gates.append(res[0:8, 0:128])
            kk = res.astype(bf16)
            k32 = pltpu.bitcast(kk, jnp.int32)
            for g in range(4):
                k_ref[g, pl.ds(r0 // 2, MQ // 2), :] = k32[:, g * 128:(g + 1) * 128]
            if (r0 + MQ) % (2 * CK) == 0:
                c0 = 2 * (r0 // (2 * CK))
                kf_ref[pl.ds(c0, 2)] = kk[MQ - 16:MQ].astype(f32).reshape(2, 8, D)
                jobs.extend((c, g, lane) for c in (c0, c0 + 1) for g in range(4) for lane in range(128))

    def proj_qv(i):
        rows = pl.ds(i * TA, TA)
        for mb in range(2 * D // MQ):
            r0 = mb * MQ
            wt = paced(wt_ref[pl.ds(r0, MQ), :], True)
            res = lax.dot_general(wt, ln1_ref[rows, :], NT, preferred_element_type=f32)
            gates.append(res[0:8, 0:128])
            if r0 < D:
                qt = (res * QSCALE).astype(bf16)
                qf_ref[pl.ds(i * H + r0 // DH, MQ // DH)] = qt.astype(f32).reshape(MQ // DH, DH, TA)
                qt_ref[i, r0 // 128, pl.ds(r0 % 128, MQ), :] = qt
            else:
                vt_ref[pl.ds((r0 - D) // DH, MQ // DH), :, rows] = (
                    pltpu.bitcast(res.astype(bf16), jnp.int32).reshape(MQ // DH, DH // 2, TA))

    x_copy(0).wait()
    ln1(0)
    wqkv_copy(1).wait()
    proj_k(0, 3)
    x_copy(1).wait()
    x_copy(2).wait()
    proj_k(3, 4)
    ln1(1)
    ln1(2, pin=True)
    proj_k(4, 9, pin_lo=6)
    x_copy(3).wait()
    wqkv_copy(0).wait()
    wqkv_copy(2).wait()
    wo_copy.start()
    for c in late_copies:
        c.start()
    proj_k(9, 12)
    ln1(3)
    proj_k(12, 16)
    wt_ref[0:D, :] = wq_ref[...].T
    wt_ref[D:2 * D, :] = wv_ref[...].T
    for i in range(NA):
        proj_qv(i)
    assert not jobs
    wo_copy.wait()

    def qm_for(t0, hl):
        t = t0 + hl
        qb = t >> 5
        g = (t >> 3) & 3
        j = hl % 8
        parts = []
        if j > 0:
            parts.append(jnp.zeros((DH * j, TQ), bf16))
        parts.append(qt_ref[qb, g, j * DH:(j + 1) * DH, :])
        if j < 7:
            parts.append(jnp.zeros((DH * (7 - j), TQ), bf16))
        return jnp.concatenate(parts, axis=0), g

    def slot(n):
        sl = n % (2 * NCK)
        return srefs[sl // 8], (sl % 8) * CK

    def run(t0, n_hi, n_qk, ms, l, acc, extra=None):
        z = z_ref[0]
        ms = dict(ms)
        mx_hist = []
        mx = None
        mv = None
        for n in range(n_hi):
            if extra is not None:
                extra(n)
            if n < n_qk:
                hl, c = divmod(n, NCK)
                if c == 0:
                    qm, g = qm_for(t0, hl)
                sref, off = slot(n)
                nm = CK - 16 if c % 2 == 1 else CK
                t = t0 + hl
                kbs = [kb_ref[t & (H - 1), c, d] for d in range(DH)]
                cols = []
                for cc in range(TQ // 128):
                    parts = [None, None]
                    for d in range(DH):
                        term = kbs[d] * qf_ref[t, pl.ds(d, 1), cc * 128:(cc + 1) * 128]
                        parts[d % 2] = term if d < 2 else parts[d % 2] + term
                    cols.append(parts[0] + parts[1])
                sv = jnp.concatenate(cols, axis=1)
                sref2, off2 = slot(n | 1)
                sref2[pl.ds(off2 + CK - 16 + 8 * (c % 2), 8), :] = sv
                mv = sv if c == 0 else jnp.maximum(mv, sv)
                k32 = k_ref[g, pl.ds(c * CK // 2, nm // 2), :]
                tiles = [k32[8 * u:8 * (u + 1)] for u in range(nm // 16)]
                for cc, u in enumerate(PINT):
                    tiles[u] = jnp.where(mv[:, cc * 128:(cc + 1) * 128] < NEG_BIG, 0, tiles[u])
                kc = pltpu.bitcast(jnp.concatenate(tiles, axis=0), bf16)
                s = jnp.dot(kc, qm, preferred_element_type=f32)
                sref[pl.ds(off, nm), :] = s
                s3 = s.reshape(nm // 8, 8, TQ)
                for r in range(nm // 8):
                    mx = s3[r] if (c == 0 and r == 0) else jnp.maximum(mx, s3[r])
                mx_hist.append(mx)
                if c == NCK - 1:
                    ms[hl] = jnp.broadcast_to(jnp.max(jnp.maximum(mx, mv), axis=0, keepdims=True), (8, TQ))
            hj, cj = divmod(n - DLAG, NCK)
            tj = t0 + hj
            h = tj & (H - 1)
            sref, off = slot(n - DLAG)
            drows = pl.ds(pl.multiple_of(off + z, CK), CK)
            m_eff = ms[hj]
            if n < n_qk and len(mx_hist) > LAGM:
                m_eff = jnp.maximum(m_eff, jnp.minimum(mx_hist[-1 - LAGM], NEG_BIG))
            p = jnp.exp2(sref[drows, :].reshape(CK // 8, 8, TQ) - m_eff[None])
            for r in range(CK // 8 - 2, -1, -2):
                pr = p[r + 1] + p[r]
                l = pr if (cj == 0 and r == CK // 8 - 2) else l + pr
            vt = pltpu.bitcast(vt_ref[h, :, pl.ds(cj * CK, CK)], bf16)
            p2 = p.reshape(CK, TQ)
            o = jnp.concatenate(
                [lax.dot_general(vt, p2[:, :PSPLIT].astype(bf16), NN, preferred_element_type=f32),
                 lax.dot_general(vt, p2[:, PSPLIT:], NN, preferred_element_type=f32)], axis=1)
            acc = o if cj == 0 else acc + o
            if cj == NCK - 1:
                lsum = jnp.sum(l, axis=0, keepdims=True)
                ot_ref[tj + 2] = (acc * (1.0 / lsum)).astype(bf16)
        return ms, l, acc

    def body(i, carry):
        ma, mb, l, acc = carry
        ms, l, acc = run(HPB * i, NCK * HPB, NCK * HPB, {-2: ma, -1: mb}, l, acc)
        return ms[HPB - 2], ms[HPB - 1], l, acc

    zeros8 = jnp.zeros((8, TQ), f32)
    ma, mb, l, acc = lax.fori_loop(0, TOTAL // HPB, body,
                                   (zeros8, zeros8, zeros8 + 1.0, jnp.zeros((DH, TQ), f32)))

    for c in late_copies:
        c.wait()

    def out_copy(i):
        return pltpu.make_async_copy(o_ref.at[pl.ds(i * TO, TO)], out_hbm.at[pl.ds(i * TO, TO)], sems.at[5])

    wr_row = wr_ref[...].reshape(1, D).astype(f32)
    wr_sum = jnp.sum(wr_row, axis=-1, keepdims=True)
    attn = {}
    deps = {}
    best = []
    int_min = jnp.iinfo(jnp.int32).min
    lane8 = lax.broadcasted_iota(jnp.int32, (8, 128), 1)
    row8 = lax.broadcasted_iota(jnp.int32, (8, 128), 0)

    def make_key(r, ids):
        bits = pltpu.bitcast(r.astype(bf16).astype(f32) + 0.0, jnp.int32)
        return jnp.where(bits >= 0, bits, bits ^ jnp.int32(0x7FFF0000)) | (S - 1 - ids)

    def insert(key):
        if not best:
            best.extend([key, jnp.full((8, 128), int_min, jnp.int32)])
        else:
            lo = jnp.minimum(best[0], key)
            best[0] = jnp.maximum(best[0], key)
            best[1] = jnp.maximum(best[1], lo)

    def all_max(v):
        return jnp.broadcast_to(jnp.max(jnp.max(v, axis=0, keepdims=True), axis=1, keepdims=True), (1, 128))

    def c_proj(i):
        qb, part = divmod(i, TQ // TC)
        o_nat = ot_ref[pl.ds(2 + qb * H, H), :, pl.ds(part * TC, TC)].reshape(D, TC).T
        if i - PINC in deps:
            zero = jnp.where(jnp.concatenate(deps.pop(i - PINC), axis=0) < NEG_BIG, -1, 0)
            head = pltpu.bitcast(pltpu.bitcast(o_nat[:, 0:128], jnp.int32) | zero, bf16)
            o_nat = jnp.concatenate([head, o_nat[:, 128:]], axis=1)
        if i == 1:
            wo32_ref[...] = pltpu.bitcast(wo_ref[...], jnp.int32)
        wo = wo_ref[...] if i == 0 else pltpu.bitcast(wo32_ref[...], bf16)
        attn[i] = jnp.dot(o_nat, wo, preferred_element_type=f32)

    def c_norm(i):
        rows = pl.ds(i * TC, TC)
        hh = x_ref[rows, :].astype(f32) + attn.pop(i)
        m, rstd = _ln_stats(hh)
        ln2 = (hh - m) * rstd
        ln2_ref[rows, :] = ln2.astype(bf16)
        o_ref[rows, :] = (hh + ln2).astype(bf16)
        if ((i + 1) * TC) % TO == 0:
            out_copy((i * TC) // TO).start()
        r = jnp.broadcast_to((jnp.sum(hh * wr_row, axis=-1, keepdims=True) - m * wr_sum) * rstd, (TC, 128))
        if i < NC - NTAIL:
            rc = r[0:8]
            for u in range(1, TC // 8):
                rc = jnp.where(lane8 == u, r[8 * u:8 * (u + 1)], rc)
                if u % 2 == 1:
                    deps.setdefault(i, []).append(rc)
            insert(jnp.where(lane8 < TC // 8, make_key(rc, i * TC + 8 * lane8 + row8), int_min))
            if i == NC - NTAIL - 1:
                k1 = all_max(best[0])
                k2 = all_max(jnp.where(best[0] == k1, best[1], best[0]))
                best[0] = jnp.where(row8 == 0, k1, int_min)
                best[1] = jnp.where(row8 == 0, k2, int_min)
        else:
            for u in range(TC // 8):
                insert(make_key(r[8 * u:8 * (u + 1)], i * TC + 8 * u + row8))

    n_early = (NQ - 1) * (TQ // TC) - NCOVER

    def c_step(i):
        if i < NC:
            c_proj(i)
        if i >= 1:
            c_norm(i - 1)

    def extra(n):
        for i in range(n * n_early // DLAG, (n + 1) * n_early // DLAG):
            c_step(i)

    run(TOTAL, DLAG, 0, {-2: ma, -1: mb}, l, acc, extra=extra)
    for i in range(n_early, NC + 1):
        c_step(i)

    k1 = jnp.max(best[0], axis=0, keepdims=True)
    k2 = jnp.max(jnp.where(best[0] == k1, best[1], best[0]), axis=0, keepdims=True)
    idxs = [S - 1 - (k[0, 0] & (S - 1)) for k in (k1, k2)]
    bases = [pl.multiple_of((idx >> 4) << 4, 16) for idx in idxs]

    xsb = jnp.concatenate([ln2_ref[pl.ds(base, 16), :] for base in bases], axis=0)
    gate = jnp.dot(xsb, wg_ref[...], preferred_element_type=f32)
    up = jnp.dot(xsb, wu_ref[...], preferred_element_type=f32)
    act = (gate * jax.nn.sigmoid(gate) * up).astype(bf16)
    y = jnp.dot(act, wd_ref[...], preferred_element_type=f32)
    rid16 = lax.broadcasted_iota(jnp.int32, (16, D), 0)
    upds = []
    for c, (k, idx, base) in enumerate(zip((k1, k2), idxs, bases)):
        kv = k & jnp.int32(-65536)
        rsel = pltpu.bitcast(jnp.where(kv >= 0, kv, kv ^ jnp.int32(0x7FFF0000)), f32)
        gatew = jnp.concatenate([jax.nn.sigmoid(rsel)] * (D // 128), axis=1)
        upds.append(jnp.where(rid16 == idx - base, y[16 * c:16 * (c + 1)] * gatew, 0.0))
    for i in range(NO):
        out_copy(i).wait()
    for upd, base in zip(upds, bases):
        o_ref[pl.ds(base, 16), :] = (o_ref[pl.ds(base, 16), :].astype(f32) + upd).astype(bf16)

    def fix_copy(c):
        return pltpu.make_async_copy(o_ref.at[pl.ds(bases[c], 16)], out_hbm.at[pl.ds(bases[c], 16)], sems.at[c])

    fix_copy(0).start()

    @pl.when(bases[0] != bases[1])
    def _():
        fix_copy(1).start()
        fix_copy(1).wait()

    fix_copy(0).wait()


@jax.jit
def pallas_sequential_preLN__mha_block__moe_arch_mod__prompt_kernel(
    A_x: jax.Array,
    A_wqkv: jax.Array,
    A_wo: jax.Array,
    B_x: jax.Array,
    B_w_r: jax.Array,
    B_w_gate: jax.Array,
    B_w_up: jax.Array,
    B_w_down: jax.Array,
):
    del B_x
    any_spec = pl.BlockSpec(memory_space=pl.ANY)
    out = pl.pallas_call(
        _kernel,
        out_shape=jax.ShapeDtypeStruct((S, D), bf16),
        in_specs=[any_spec] * 7,
        out_specs=any_spec,
        scratch_shapes=[
            pltpu.VMEM((S, D), bf16),
            pltpu.VMEM((D, D), bf16),
            pltpu.VMEM((D, D), bf16),
            pltpu.VMEM((D, D), bf16),
            pltpu.VMEM((D, D), bf16),
            pltpu.VMEM((D // 2, D), jnp.int32),
            pltpu.VMEM((D,), bf16),
            pltpu.VMEM((D, F), bf16),
            pltpu.VMEM((D, F), bf16),
            pltpu.VMEM((F, D), bf16),
            pltpu.VMEM((2 * D, D), bf16),
            pltpu.VMEM((S, D), bf16),
            pltpu.VMEM((4, S // 2, 128), jnp.int32),
            pltpu.VMEM((NQ, 4, 128, TQ), bf16),
            pltpu.VMEM((H, DH // 2, S), jnp.int32),
            pltpu.VMEM((TOTAL + 2, DH, TQ), bf16),
            pltpu.VMEM((NCK, 8, D), f32),
            pltpu.VMEM((H, NCK, DH, 8, 128), f32),
            pltpu.VMEM((TOTAL, DH, TQ), f32),
            pltpu.VMEM((8 * CK, TQ), f32),
            pltpu.VMEM((8 * CK, TQ), f32),
            pltpu.VMEM((8 * CK, TQ), f32),
            pltpu.VMEM((8 * CK, TQ), f32),
            pltpu.VMEM((S, D), bf16),
            pltpu.VMEM((S, D), bf16),
            pltpu.SMEM((1,), jnp.int32),
            pltpu.SemaphoreType.DMA((6,)),
        ],
        compiler_params=pltpu.CompilerParams(vmem_limit_bytes=110 * 1024 * 1024),
    )(A_x.reshape(S, D), A_wqkv, A_wo, B_w_r, B_w_gate, B_w_up, B_w_down)
    return out.reshape(1, S, D)
```

```python
import jax
import jax.numpy as jnp
from jax import lax
import jax.experimental.pallas as pl
import jax.experimental.pallas.tpu as pltpu

S = 2048
D = 512
H = 32
DH = 16
F = 1792
EPS = 1e-5
QSCALE = (DH ** -0.5) * 1.4426950408889634

TA = 512
NA = S // TA
MQ = 128
TQ = 512
NQ = S // TQ
TOTAL = H * NQ
HPB = 8
CK = 128
NCK = S // CK
DLAG = NCK + 2
TC = 128
NC = S // TC
TO = 256
NO = S // TO

NEG_BIG = -3.0e38
LAGM = 3
PINT = (4, 5, 6, 6)
PSPLIT = 384
KB_PER_TILE = (0, 8, 16, 8)
GLAG = 2
PINC = 3
NTAIL = 2
NCOVER = 1

f32 = jnp.float32
bf16 = jnp.bfloat16
NN = (((1,), (0,)), ((), ()))
NT = (((1,), (1,)), ((), ()))


def _ln_stats(x):
    m = jnp.sum(x, axis=-1, keepdims=True) * (1.0 / D)
    v = jnp.maximum(jnp.sum(x * x, axis=-1, keepdims=True) * (1.0 / D) - m * m, 0.0)
    return m, lax.rsqrt(v + EPS)


def _layernorm(x):
    m = jnp.mean(x, axis=-1, keepdims=True)
    xc = x - m
    v = jnp.mean(xc * xc, axis=-1, keepdims=True)
    return xc * lax.rsqrt(v + EPS)


def _kernel(x_hbm, wqkv_hbm, wo_hbm, wr_hbm, wg_hbm, wu_hbm, wd_hbm, out_hbm,
            x_ref, wq_ref, wk_ref, wv_ref, wo_ref, wo32_ref, wr_ref, wg_ref, wu_ref, wd_ref, wt_ref, ln1_ref,
            k_ref, qt_ref, vt_ref, ot_ref, kf_ref, kb_ref, qf_ref, s0, s1, s2, s3,
            ln2_ref, o_ref, z_ref, sems):
    srefs = [s0, s1, s2, s3]

    def x_copy(i):
        return pltpu.make_async_copy(x_hbm.at[pl.ds(i * TA, TA)], x_ref.at[pl.ds(i * TA, TA)],
                                     sems.at[(0, 2, 2, 3)[i]])

    def wqkv_copy(part):
        return pltpu.make_async_copy(wqkv_hbm.at[:, pl.ds(part * D, D)], (wq_ref, wk_ref, wv_ref)[part],
                                     sems.at[(3, 1, 3)[part]])

    wo_copy = pltpu.make_async_copy(wo_hbm, wo_ref, sems.at[0])
    late_copies = [
        pltpu.make_async_copy(wr_hbm, wr_ref, sems.at[4]),
        pltpu.make_async_copy(wg_hbm, wg_ref, sems.at[4]),
        pltpu.make_async_copy(wu_hbm, wu_ref, sems.at[4]),
        pltpu.make_async_copy(wd_hbm, wd_ref, sems.at[4]),
    ]
    x_copy(0).start()
    wqkv_copy(1).start()
    for i in range(1, NA):
        x_copy(i).start()
    wqkv_copy(0).start()
    wqkv_copy(2).start()
    z_ref[0] = 0
    for sl in range(2 * NCK - DLAG, 2 * NCK):
        srefs[sl // 8][pl.ds((sl % 8) * CK, CK), :] = jnp.zeros((CK, TQ), f32)

    ln_deps = []

    def ln1(i, pin=False):
        rows = pl.ds(i * TA, TA)
        ln = _layernorm(x_ref[rows, :].astype(f32))
        ln1_ref[rows, :] = ln.astype(bf16)
        if pin:
            for u in range(TA // 8):
                row = ln[8 * u:8 * (u + 1)]
                ln_deps.append(jnp.minimum(jnp.minimum(row[:, 0:128], row[:, 128:256]),
                                           jnp.minimum(row[:, 256:384], row[:, 384:512])))

    jobs = []
    gates = []

    def paced(lhs, with_jobs, n_deps=0):
        if not with_jobs and n_deps == 0:
            return lhs
        n_tiles = (lhs.shape[0] // 16) * (lhs.shape[1] // 128)
        tile_no = 0
        w32 = pltpu.bitcast(lhs, jnp.int32)
        gate = gates[-GLAG] if len(gates) >= GLAG else None
        cols = []
        for kt in range(w32.shape[1] // 128):
            tiles = []
            for u in range(w32.shape[0] // 8):
                tile = w32[8 * u:8 * (u + 1), kt * 128:(kt + 1) * 128]
                lo = None
                src = {}
                tile_no += 1
                for _ in range(n_deps * tile_no // n_tiles - n_deps * (tile_no - 1) // n_tiles):
                    dep = ln_deps.pop(0)
                    lo = dep if lo is None else jnp.minimum(lo, dep)
                for _ in range(KB_PER_TILE[kt] if with_jobs else 0):
                    c, g, lane = jobs.pop(0)
                    if (c, g) not in src:
                        src[c, g] = jnp.where(gate < NEG_BIG, 0.0, kf_ref[c, :, g * 128:(g + 1) * 128])
                    kb = jnp.broadcast_to(src[c, g][:, lane:lane + 1], (8, 128))
                    col = g * 128 + lane
                    kb_ref[col // DH, c, col % DH] = kb
                    lo = kb if lo is None else jnp.minimum(lo, kb)
                tiles.append(tile if lo is None else jnp.where(lo < NEG_BIG, 0, tile))
            cols.append(jnp.concatenate(tiles, axis=0))
        return pltpu.bitcast(jnp.concatenate(cols, axis=1), bf16)

    def proj_k(lo, hi, pin_lo=None):
        for mb in range(lo, hi):
            r0 = mb * MQ
            rows = pl.ds(r0, MQ)
            n_deps = -(-len(ln_deps) // (hi - mb)) if (pin_lo is not None and mb >= pin_lo) else 0
            res = jnp.dot(paced(ln1_ref[rows, :], False, n_deps), wk_ref[...], preferred_element_type=f32)
            gates.append(res[0:8, 0:128])
            kk = res.astype(bf16)
            k32 = pltpu.bitcast(kk, jnp.int32)
            for g in range(4):
                k_ref[g, pl.ds(r0 // 2, MQ // 2), :] = k32[:, g * 128:(g + 1) * 128]
            if (r0 + MQ) % (2 * CK) == 0:
                c0 = 2 * (r0 // (2 * CK))
                kf_ref[pl.ds(c0, 2)] = kk[MQ - 16:MQ].astype(f32).reshape(2, 8, D)
                jobs.extend((c, g, lane) for c in (c0, c0 + 1) for g in range(4) for lane in range(128))

    def proj_qv(i):
        rows = pl.ds(i * TA, TA)
        for mb in range(2 * D // MQ):
            r0 = mb * MQ
            wt = paced(wt_ref[pl.ds(r0, MQ), :], True)
            res = lax.dot_general(wt, ln1_ref[rows, :], NT, preferred_element_type=f32)
            gates.append(res[0:8, 0:128])
            if r0 < D:
                qt = (res * QSCALE).astype(bf16)
                qf_ref[pl.ds(i * H + r0 // DH, MQ // DH)] = qt.astype(f32).reshape(MQ // DH, DH, TA)
                qt_ref[i, r0 // 128, pl.ds(r0 % 128, MQ), :] = qt
            else:
                vt_ref[pl.ds((r0 - D) // DH, MQ // DH), :, rows] = (
                    pltpu.bitcast(res.astype(bf16), jnp.int32).reshape(MQ // DH, DH // 2, TA))

    x_copy(0).wait()
    ln1(0)
    wqkv_copy(1).wait()
    proj_k(0, 3)
    x_copy(1).wait()
    x_copy(2).wait()
    proj_k(3, 4)
    ln1(1)
    ln1(2, pin=True)
    proj_k(4, 9, pin_lo=6)
    x_copy(3).wait()
    wqkv_copy(0).wait()
    wqkv_copy(2).wait()
    wo_copy.start()
    for c in late_copies:
        c.start()
    proj_k(9, 12)
    ln1(3)
    proj_k(12, 16)
    wt_ref[0:D, :] = wq_ref[...].T
    wt_ref[D:2 * D, :] = wv_ref[...].T
    for i in range(NA):
        proj_qv(i)
    assert not jobs
    wo_copy.wait()

    def qm_for(t, j):
        qb = t >> 5
        g = (t >> 3) & 3
        parts = []
        if j > 0:
            parts.append(jnp.zeros((DH * j, TQ), bf16))
        parts.append(qt_ref[qb, g, j * DH:(j + 1) * DH, :])
        if j < 7:
            parts.append(jnp.zeros((DH * (7 - j), TQ), bf16))
        return jnp.concatenate(parts, axis=0), g

    def slot(n):
        sl = n % (2 * NCK)
        return srefs[sl // 8], (sl % 8) * CK

    def run(t0, n_hi, n_qk, ms, l, acc, extra=None):
        z = z_ref[0]
        ms = dict(ms)
        mx_hist = []
        mx = None
        mv = None
        for n in range(n_hi):
            if extra is not None:
                extra(n)
            if n < n_qk:
                hl, c = divmod(n, NCK)
                if c == 0:
                    t = t0 + hl
                    head = t & (H - 1)
                    qm, g = qm_for(t, hl % 8)
                sref, off = slot(n)
                nm = CK - 16 if c % 2 == 1 else CK
                kbs = [kb_ref[head, c, d] for d in range(DH)]
                cols = []
                for cc in range(TQ // 128):
                    parts = [None, None]
                    for d in range(DH):
                        term = kbs[d] * qf_ref[t, pl.ds(d, 1), cc * 128:(cc + 1) * 128]
                        parts[d % 2] = term if d < 2 else parts[d % 2] + term
                    cols.append(parts[0] + parts[1])
                sv = jnp.concatenate(cols, axis=1)
                sref2, off2 = slot(n | 1)
                sref2[pl.ds(off2 + CK - 16 + 8 * (c % 2), 8), :] = sv
                mv = sv if c == 0 else jnp.maximum(mv, sv)
                k32 = k_ref[g, pl.ds(c * CK // 2, nm // 2), :]
                tiles = [k32[8 * u:8 * (u + 1)] for u in range(nm // 16)]
                for cc, u in enumerate(PINT):
                    tiles[u] = jnp.where(mv[:, cc * 128:(cc + 1) * 128] < NEG_BIG, 0, tiles[u])
                kc = pltpu.bitcast(jnp.concatenate(tiles, axis=0), bf16)
                s = jnp.dot(kc, qm, preferred_element_type=f32)
                sref[pl.ds(off, nm), :] = s
                s3 = s.reshape(nm // 8, 8, TQ)
                mx = jnp.max(s3 if c == 0 else jnp.concatenate([mx[None], s3], axis=0), axis=0)
                mx_hist.append(mx)
                if c == NCK - 1:
                    ms[hl] = jnp.broadcast_to(jnp.max(jnp.maximum(mx, mv), axis=0, keepdims=True), (8, TQ))
            hj, cj = divmod(n - DLAG, NCK)
            tj = t0 + hj
            h = tj & (H - 1)
            sref, off = slot(n - DLAG)
            drows = pl.ds(pl.multiple_of(off + z, CK), CK)
            m_eff = ms[hj]
            if n < n_qk and len(mx_hist) > LAGM:
                m_eff = jnp.maximum(m_eff, jnp.minimum(mx_hist[-1 - LAGM], NEG_BIG))
            p2 = jnp.exp2(sref[drows, :].reshape(CK // 8, 8, TQ) - m_eff[None]).reshape(CK, TQ)
            for r in range(CK - 16, -1, -16):
                pr = p2[r + 8:r + 16] + p2[r:r + 8]
                l = pr if (cj == 0 and r == CK - 16) else l + pr
            vt = pltpu.bitcast(vt_ref[h, :, pl.ds(cj * CK, CK)], bf16)
            o = jnp.concatenate(
                [lax.dot_general(vt, p2[:, :PSPLIT].astype(bf16), NN, preferred_element_type=f32),
                 lax.dot_general(vt, p2[:, PSPLIT:], NN, preferred_element_type=f32)], axis=1)
            acc = o if cj == 0 else acc + o
            if cj == NCK - 1:
                lsum = jnp.sum(l, axis=0, keepdims=True)
                ot_ref[tj + 2] = (acc * (1.0 / lsum)).astype(bf16)
        return ms, l, acc

    def body(i, carry):
        ma, mb, l, acc = carry
        ms, l, acc = run(HPB * i, NCK * HPB, NCK * HPB, {-2: ma, -1: mb}, l, acc)
        return ms[HPB - 2], ms[HPB - 1], l, acc

    zeros8 = jnp.zeros((8, TQ), f32)
    ma, mb, l, acc = lax.fori_loop(0, TOTAL // HPB, body,
                                   (zeros8, zeros8, zeros8 + 1.0, jnp.zeros((DH, TQ), f32)))

    for c in late_copies:
        c.wait()

    def out_copy(i):
        return pltpu.make_async_copy(o_ref.at[pl.ds(i * TO, TO)], out_hbm.at[pl.ds(i * TO, TO)], sems.at[5])

    wr_row = wr_ref[...].reshape(1, D).astype(f32)
    wr_sum = jnp.sum(wr_row, axis=-1, keepdims=True)
    attn = {}
    deps = {}
    best = []
    int_min = jnp.iinfo(jnp.int32).min
    lane8 = lax.broadcasted_iota(jnp.int32, (8, 128), 1)
    row8 = lax.broadcasted_iota(jnp.int32, (8, 128), 0)

    def make_key(r, ids):
        bits = pltpu.bitcast(r.astype(bf16).astype(f32) + 0.0, jnp.int32)
        return jnp.where(bits >= 0, bits, bits ^ jnp.int32(0x7FFF0000)) | (S - 1 - ids)

    def insert(key):
        if not best:
            best.extend([key, jnp.full((8, 128), int_min, jnp.int32)])
        else:
            lo = jnp.minimum(best[0], key)
            best[0] = jnp.maximum(best[0], key)
            best[1] = jnp.maximum(best[1], lo)

    def all_max(v):
        return jnp.broadcast_to(jnp.max(jnp.max(v, axis=0, keepdims=True), axis=1, keepdims=True), (1, 128))

    def c_proj(i):
        qb, part = divmod(i, TQ // TC)
        o_nat = ot_ref[pl.ds(2 + qb * H, H), :, pl.ds(part * TC, TC)].reshape(D, TC).T
        if i - PINC in deps:
            zero = jnp.where(jnp.concatenate(deps.pop(i - PINC), axis=0) < NEG_BIG, -1, 0)
            head = pltpu.bitcast(pltpu.bitcast(o_nat[:, 0:128], jnp.int32) | zero, bf16)
            o_nat = jnp.concatenate([head, o_nat[:, 128:]], axis=1)
        if i == 1:
            wo32_ref[...] = pltpu.bitcast(wo_ref[...], jnp.int32)
        wo = wo_ref[...] if i == 0 else pltpu.bitcast(wo32_ref[...], bf16)
        attn[i] = jnp.dot(o_nat, wo, preferred_element_type=f32)

    def c_norm(i):
        rows = pl.ds(i * TC, TC)
        hh = x_ref[rows, :].astype(f32) + attn.pop(i)
        m, rstd = _ln_stats(hh)
        ln2 = (hh - m) * rstd
        ln2_ref[rows, :] = ln2.astype(bf16)
        o_ref[rows, :] = (hh + ln2).astype(bf16)
        if ((i + 1) * TC) % TO == 0:
            out_copy((i * TC) // TO).start()
        r = jnp.broadcast_to((jnp.sum(hh * wr_row, axis=-1, keepdims=True) - m * wr_sum) * rstd, (TC, 128))
        if i < NC - NTAIL:
            rc = r[0:8]
            for u in range(1, TC // 8):
                rc = jnp.where(lane8 == u, r[8 * u:8 * (u + 1)], rc)
                if u % 2 == 1:
                    deps.setdefault(i, []).append(rc)
            insert(jnp.where(lane8 < TC // 8, make_key(rc, i * TC + 8 * lane8 + row8), int_min))
            if i == NC - NTAIL - 1:
                k1 = all_max(best[0])
                k2 = all_max(jnp.where(best[0] == k1, best[1], best[0]))
                best[0] = jnp.where(row8 == 0, k1, int_min)
                best[1] = jnp.where(row8 == 0, k2, int_min)
        else:
            for u in range(TC // 8):
                insert(make_key(r[8 * u:8 * (u + 1)], i * TC + 8 * u + row8))

    n_early = (NQ - 1) * (TQ // TC) - NCOVER

    def c_step(i):
        if i < NC:
            c_proj(i)
        if i >= 1:
            c_norm(i - 1)

    def extra(n):
        for i in range(n * n_early // DLAG, (n + 1) * n_early // DLAG):
            c_step(i)

    run(TOTAL, DLAG, 0, {-2: ma, -1: mb}, l, acc, extra=extra)
    for i in range(n_early, NC + 1):
        c_step(i)

    k1 = jnp.max(best[0], axis=0, keepdims=True)
    k2 = jnp.max(jnp.where(best[0] == k1, best[1], best[0]), axis=0, keepdims=True)
    idxs = [S - 1 - (k[0, 0] & (S - 1)) for k in (k1, k2)]
    bases = [pl.multiple_of((idx >> 4) << 4, 16) for idx in idxs]

    xsb = jnp.concatenate([ln2_ref[pl.ds(base, 16), :] for base in bases], axis=0)
    gate = jnp.dot(xsb, wg_ref[...], preferred_element_type=f32)
    up = jnp.dot(xsb, wu_ref[...], preferred_element_type=f32)
    act = (gate * jax.nn.sigmoid(gate) * up).astype(bf16)
    y = jnp.dot(act, wd_ref[...], preferred_element_type=f32)
    rid16 = lax.broadcasted_iota(jnp.int32, (16, D), 0)
    upds = []
    for c, (k, idx, base) in enumerate(zip((k1, k2), idxs, bases)):
        kv = k & jnp.int32(-65536)
        rsel = pltpu.bitcast(jnp.where(kv >= 0, kv, kv ^ jnp.int32(0x7FFF0000)), f32)
        gatew = jnp.concatenate([jax.nn.sigmoid(rsel)] * (D // 128), axis=1)
        upds.append(jnp.where(rid16 == idx - base, y[16 * c:16 * (c + 1)] * gatew, 0.0))
    for i in range(NO):
        out_copy(i).wait()
    for upd, base in zip(upds, bases):
        o_ref[pl.ds(base, 16), :] = (o_ref[pl.ds(base, 16), :].astype(f32) + upd).astype(bf16)

    def fix_copy(c):
        return pltpu.make_async_copy(o_ref.at[pl.ds(bases[c], 16)], out_hbm.at[pl.ds(bases[c], 16)], sems.at[c])

    fix_copy(0).start()

    @pl.when(bases[0] != bases[1])
    def _():
        fix_copy(1).start()
        fix_copy(1).wait()

    fix_copy(0).wait()


@jax.jit
def pallas_sequential_preLN__mha_block__moe_arch_mod__prompt_kernel(
    A_x: jax.Array,
    A_wqkv: jax.Array,
    A_wo: jax.Array,
    B_x: jax.Array,
    B_w_r: jax.Array,
    B_w_gate: jax.Array,
    B_w_up: jax.Array,
    B_w_down: jax.Array,
):
    del B_x
    any_spec = pl.BlockSpec(memory_space=pl.ANY)
    out = pl.pallas_call(
        _kernel,
        out_shape=jax.ShapeDtypeStruct((S, D), bf16),
        in_specs=[any_spec] * 7,
        out_specs=any_spec,
        scratch_shapes=[
            pltpu.VMEM((S, D), bf16),
            pltpu.VMEM((D, D), bf16),
            pltpu.VMEM((D, D), bf16),
            pltpu.VMEM((D, D), bf16),
            pltpu.VMEM((D, D), bf16),
            pltpu.VMEM((D // 2, D), jnp.int32),
            pltpu.VMEM((D,), bf16),
            pltpu.VMEM((D, F), bf16),
            pltpu.VMEM((D, F), bf16),
            pltpu.VMEM((F, D), bf16),
            pltpu.VMEM((2 * D, D), bf16),
            pltpu.VMEM((S, D), bf16),
            pltpu.VMEM((4, S // 2, 128), jnp.int32),
            pltpu.VMEM((NQ, 4, 128, TQ), bf16),
            pltpu.VMEM((H, DH // 2, S), jnp.int32),
            pltpu.VMEM((TOTAL + 2, DH, TQ), bf16),
            pltpu.VMEM((NCK, 8, D), f32),
            pltpu.VMEM((H, NCK, DH, 8, 128), f32),
            pltpu.VMEM((TOTAL, DH, TQ), f32),
            pltpu.VMEM((8 * CK, TQ), f32),
            pltpu.VMEM((8 * CK, TQ), f32),
            pltpu.VMEM((8 * CK, TQ), f32),
            pltpu.VMEM((8 * CK, TQ), f32),
            pltpu.VMEM((S, D), bf16),
            pltpu.VMEM((S, D), bf16),
            pltpu.SMEM((1,), jnp.int32),
            pltpu.SemaphoreType.DMA((6,)),
        ],
        compiler_params=pltpu.CompilerParams(vmem_limit_bytes=110 * 1024 * 1024),
    )(A_x.reshape(S, D), A_wqkv, A_wo, B_w_r, B_w_gate, B_w_up, B_w_down)
    return out.reshape(1, S, D)
```
